```python
import os as _os
_os.environ.setdefault("JAX_PLATFORMS", "cpu")
import jax
import jax.numpy as jnp

def _softmax(x, axis=-1):
    return jax.nn.softmax(x, axis=axis)
def _gelu(x):
    return jax.nn.gelu(x, approximate=True)
def _silu(x):
    return jax.nn.silu(x)
def _sigmoid(x):
    return jax.nn.sigmoid(x)
def _layernorm(x, axis=-1, eps=1e-5):
    m = jnp.mean(x, axis=axis, keepdims=True)
    v = jnp.var(x, axis=axis, keepdims=True)
    return (x - m) / jnp.sqrt(v + eps)
def _scatter_add(tgt, idx, src, axis=0):
    return tgt.at[idx].add(src)
def _segment_sum(src, seg, n):
    return jax.ops.segment_sum(src, seg, n)
class _Rng:
    def __init__(self, key):
        self._k = key
    def _next(self):
        self._k, sub = jax.random.split(self._k)
        return sub
    def normal(self, shape):
        return jax.random.normal(self._next(), shape, dtype=jnp.bfloat16)
    def randint(self, lo, hi, shape):
        return jax.random.randint(self._next(), shape, lo, hi, dtype=jnp.int32)
    def uniform(self, shape, lo=0.0, hi=1.0):
        return jax.random.uniform(self._next(), shape, jnp.bfloat16, lo, hi)
    def permutation(self, n):
        return jax.random.permutation(self._next(), n)


kernel_name = 'parallel_sum__softmax_full_mha__glu_gated_swiglu__prompt'

def setup_inputs():
    _rng = _Rng(jax.random.key(int.from_bytes(__import__("os").urandom(4), "little")))
    _w = (lambda a: (lambda t: t.astype(jnp.bfloat16) if jnp.issubdtype(t.dtype, jnp.floating) else t)(jnp.asarray(a)))
    def _A_setup():
        B, S, D = 1, 2048, 448
        return {
            "x": _w((lambda *s: _rng.normal(s) * 0.05)(B, S, D)),
            "wqkv": _w((lambda *s: _rng.normal(s) * 0.05)(D, 3 * D)),
            "wo": _w((lambda *s: _rng.normal(s) * 0.05)(D, D)),
        }
    _A_in = _A_setup()

    def _B_setup():
        B, S, D, F = 1, 2048, 448, 1792
        return {
            "x": _w((lambda *s: _rng.normal(s) * 0.05)(B, S, D)),
            "w1": _w((lambda *s: _rng.normal(s) * 0.05)(D, F) * (2.0 / D) ** 0.5),
            "w3": _w((lambda *s: _rng.normal(s) * 0.05)(D, F) * (2.0 / D) ** 0.5),
            "w2": _w((lambda *s: _rng.normal(s) * 0.05)(F, D) * (2.0 / F) ** 0.5),
        }
    _B_in = _B_setup()

    return {
        "A_x": _A_in["x"],
        "A_wqkv": _A_in["wqkv"],
        "A_wo": _A_in["wo"],
        "B_x": _B_in["x"],
        "B_w1": _B_in["w1"],
        "B_w3": _B_in["w3"],
        "B_w2": _B_in["w2"],
    }

def reference(A_x, A_wqkv, A_wo, B_x, B_w1, B_w3, B_w2):
    def _A_ref(x, wqkv, wo):
        B, S, D = x.shape
        H = 16; Dh = D // H
        qkv = (lambda x, *d: x.transpose(*d))((x @ wqkv).reshape(B, S, 3, H, Dh), 2, 0, 3, 1, 4)
        q, k, v = qkv[0], qkv[1], qkv[2]
        scale = Dh ** -0.5
        scores = jnp.einsum("bhqd,bhkd->bhqk", q, k) * scale
        p = _softmax(scores, axis=-1)
        o = jnp.einsum("bhqk,bhkd->bhqd", p, v)
        return (lambda x, *d: x.transpose(*d))(o, 0, 2, 1, 3).reshape(B, S, D) @ wo

    def _B_ref(x, w1, w3, w2):
        gate = jnp.einsum("bsd,df->bsf", x, w1)
        up = jnp.einsum("bsd,df->bsf", x, w3)
        h = _silu(gate) * up
        out = jnp.einsum("bsf,fd->bsd", h, w2)
        return out

    x = A_x
    xn = _layernorm(x, axis=-1)
    return x + _A_ref(xn, A_wqkv, A_wo) + _B_ref(xn, B_w1, B_w3, B_w2)
```

```python
import math

import jax
import jax.numpy as jnp
import jax.experimental.pallas as pl
import jax.experimental.pallas.tpu as pltpu

S = 2048
D = 448
H = 16
DH = 28
DP = 32
F = 1792
TQ = 512
NQ = S // TQ
CK = 128
NCK = S // CK
TR = 512
EPS = 1e-5
QSCALE = (DH ** -0.5) * math.log2(math.e)

F32 = jnp.float32
BF16 = jnp.bfloat16
NT = (((1,), (1,)), ((), ()))


def _kernel(x_ref, wqkv_ref, wo_ref, w1_ref, w3_ref, w2_ref, o_ref,
            wt_ref, wtmp_ref, wop_ref, xn_ref, qtm_ref, k_ref, vt_ref,
            sa, sb, ma, mb, ot_ref):
    for c in range(11):
        w = min(128, 3 * D - c * 128)
        wtmp_ref[c * 128:c * 128 + w, :] = wqkv_ref[:, c * 128:c * 128 + w].astype(F32).T
    wt_ref[...] = jnp.zeros_like(wt_ref)
    for j in range(3 * H):
        wt_ref[DP * j:DP * j + DH, :] = wtmp_ref[DH * j:DH * j + DH, :].astype(BF16)
    wtmp_ref[0:D, :] = wo_ref[...].astype(F32)
    wop_ref[...] = jnp.zeros_like(wop_ref)
    for j in range(H):
        wop_ref[DP * j:DP * j + DH, :] = wtmp_ref[DH * j:DH * j + DH, :].astype(BF16)
    qtm_ref[...] = jnp.zeros_like(qtm_ref)

    for r in range(S // TR):
        rows = slice(r * TR, (r + 1) * TR)
        x = x_ref[rows, :].astype(F32)
        mu = jnp.mean(x, axis=-1, keepdims=True)
        xc = x - mu
        var = jnp.mean(xc * xc, axis=-1, keepdims=True)
        xn = (xc * jax.lax.rsqrt(var + EPS)).astype(BF16)
        xn_ref[rows, :] = xn
        qt = jax.lax.dot_general(wt_ref[0:512, :], xn, NT, preferred_element_type=F32)
        qt = (qt * QSCALE).astype(BF16)
        for h in range(H):
            j = h % 4
            qtm_ref[r * H + h, DP * j:DP * (j + 1), :] = qt[DP * h:DP * (h + 1), :]
        kk = jax.lax.dot_general(xn, wt_ref[512:1024, :], NT, preferred_element_type=F32).astype(BF16)
        for g in range(4):
            k_ref[g, rows, :] = kk[:, 128 * g:128 * (g + 1)]
        vt = jax.lax.dot_general(wt_ref[1024:1536, :], xn, NT, preferred_element_type=F32)
        rid = jax.lax.broadcasted_iota(jnp.int32, vt.shape, 0)
        vt = jnp.where((rid % DP) == DH, 1.0, vt).astype(BF16)
        for h in range(H):
            vt_ref[h, :, rows] = vt[DP * h:DP * (h + 1), :]

    T = NQ * H

    def qk_chunk(t, c, s_ref, mrun):
        g = (t % H) // 4
        s = jnp.dot(k_ref[g, c * CK:(c + 1) * CK, :], qtm_ref[t], preferred_element_type=F32)
        s_ref[c * CK:(c + 1) * CK, :] = s
        mm = jnp.max(s.reshape(CK // 8, 8, TQ), axis=0)
        return mm if mrun is None else jnp.maximum(mrun, mm)

    def pv_chunk(t, c, s_ref, m, acc):
        h = t % H
        p = jnp.exp2(s_ref[c * CK:(c + 1) * CK, :] - m).astype(BF16)
        o = jnp.dot(vt_ref[h, :, c * CK:(c + 1) * CK], p, preferred_element_type=F32)
        return o if acc is None else acc + o

    def step(t_qk, t_pv, s_w, m_w, s_r, m_r):
        m = m_r[...]
        mrun = None
        acc = None
        for c in range(NCK):
            mrun = qk_chunk(t_qk, c, s_w, mrun)
            acc = pv_chunk(t_pv, c, s_r, m, acc)
        m_w[...] = jnp.max(mrun, axis=0, keepdims=True)
        inv = 1.0 / acc[DH:DH + 1, :]
        ot_ref[t_pv] = acc * inv

    mrun = None
    for c in range(NCK):
        mrun = qk_chunk(0, c, sa, mrun)
    ma[...] = jnp.max(mrun, axis=0, keepdims=True)

    def body(i, carry):
        t = 2 * i
        step(t + 1, t, sb, mb, sa, ma)
        step(jnp.minimum(t + 2, T - 1), t + 1, sa, ma, sb, mb)
        return carry

    jax.lax.fori_loop(0, T // 2, body, 0)

    def fin(r, carry):
        rows = pl.ds(pl.multiple_of(r * TR, TR), TR)
        xn = xn_ref[rows, :]
        g = jnp.dot(xn, w1_ref[...], preferred_element_type=F32)
        u = jnp.dot(xn, w3_ref[...], preferred_element_type=F32)
        hh = (g * jax.nn.sigmoid(g) * u).astype(BF16)
        y = jnp.dot(hh, w2_ref[...], preferred_element_type=F32)
        ot = ot_ref[pl.ds(r * H, H)].reshape(H * DP, TQ)
        o = ot.T.astype(BF16)
        y = y + jnp.dot(o, wop_ref[...], preferred_element_type=F32)
        o_ref[rows, :] = (x_ref[rows, :].astype(F32) + y).astype(o_ref.dtype)
        return carry

    jax.lax.fori_loop(0, S // TR, fin, 0)


@jax.jit
def pallas_parallel_sum__softmax_full_mha__glu_gated_swiglu__prompt_kernel(
    A_x: jax.Array,
    A_wqkv: jax.Array,
    A_wo: jax.Array,
    B_x: jax.Array,
    B_w1: jax.Array,
    B_w3: jax.Array,
    B_w2: jax.Array,
):
    del B_x
    x = A_x.reshape(S, D)
    out = pl.pallas_call(
        _kernel,
        out_shape=jax.ShapeDtypeStruct((S, D), A_x.dtype),
        scratch_shapes=[
            pltpu.VMEM((3 * H * DP, D), BF16),
            pltpu.VMEM((3 * D, D), F32),
            pltpu.VMEM((H * DP, D), BF16),
            pltpu.VMEM((S, D), BF16),
            pltpu.VMEM((NQ * H, 128, TQ), BF16),
            pltpu.VMEM((4, S, 128), BF16),
            pltpu.VMEM((H, DP, S), BF16),
            pltpu.VMEM((S, TQ), F32),
            pltpu.VMEM((S, TQ), F32),
            pltpu.VMEM((1, TQ), F32),
            pltpu.VMEM((1, TQ), F32),
            pltpu.VMEM((NQ * H, DP, TQ), F32),
        ],
        compiler_params=pltpu.CompilerParams(vmem_limit_bytes=100 * 1024 * 1024),
    )(x, A_wqkv, A_wo, B_w1, B_w3, B_w2)
    return out.reshape(1, S, D)
```

```python
import math

import jax
import jax.numpy as jnp
import jax.experimental.pallas as pl
import jax.experimental.pallas.tpu as pltpu

S = 2048
D = 448
H = 16
DH = 28
DP = 32
G = 112
F = 1792
TQ = 256
NQ = S // TQ
CK = 128
NCK = S // CK
TA = 512
NA = S // TA
FS = 2
NDP = 4
EPS = 1e-5
QSCALE = (DH ** -0.5) * math.log2(math.e)

F32 = jnp.float32
BF16 = jnp.bfloat16
U32 = jnp.uint32
NT = (((1,), (1,)), ((), ()))


def _pk(x):
    return pltpu.bitcast(x, U32)


def _upk(x):
    return pltpu.bitcast(x, BF16)


def _win(h):
    if h % 2 == 0:
        return DH * h, 0, DH
    return DH * h - 4, 4, 0


def _kernel(xt_hbm, wqkv_hbm, wo_hbm, w1_hbm, w3_hbm, w2t_hbm, o_hbm,
            xt_ref, wqkv_ref, wo_ref, w1_ref, w3_ref, w2t_ref, ob_ref, sems,
            wt_ref, wot_ref, xn_ref, qt_ref, k_ref, vt_ref,
            sa, sb, ot_ref, h_ref):
    cp_wq = pltpu.make_async_copy(wqkv_hbm.at[:, 0:512], wqkv_ref.at[:, 0:512], sems.at[0])
    cp_wkv = pltpu.make_async_copy(wqkv_hbm.at[:, 512:3 * D], wqkv_ref.at[:, 512:3 * D], sems.at[1])
    cp_wo = pltpu.make_async_copy(wo_hbm, wo_ref, sems.at[2])
    cp_w1 = pltpu.make_async_copy(w1_hbm, w1_ref, sems.at[3])
    cp_w3 = pltpu.make_async_copy(w3_hbm, w3_ref, sems.at[4])
    cp_w2 = pltpu.make_async_copy(w2t_hbm, w2t_ref, sems.at[5])
    cp_x = [pltpu.make_async_copy(xt_hbm.at[:, r * TQ:(r + 1) * TQ], xt_ref.at[r], sems.at[6 + r])
            for r in range(NQ)]
    nx0 = TA // TQ
    for c in cp_x[:nx0]:
        c.start()
    cp_wq.start()
    cp_wkv.start()
    for c in cp_x[nx0:]:
        c.start()
    cp_wo.start()
    cp_w1.start()
    cp_w3.start()
    cp_w2.start()

    def layernorm(a):
        outs = []
        for r in range(a * nx0, (a + 1) * nx0):
            for i in range(TQ // 128):
                x = xt_ref[r, :, 128 * i:128 * (i + 1)].astype(F32)
                mu = jnp.mean(x, axis=0, keepdims=True)
                xc = x - mu
                var = jnp.mean(xc * xc, axis=0, keepdims=True)
                outs.append((xc * jax.lax.rsqrt(var + EPS)).astype(BF16))
        return jnp.concatenate(outs, axis=1)

    def store_xn(a, xnt):
        xn_ref[a * TA // 2:(a + 1) * TA // 2, :] = _pk(xnt.T)

    def proj_q(a, xnt):
        qt = jnp.dot(_upk(wt_ref[0:D // 2, :]), xnt, preferred_element_type=F32)
        qt = _pk((qt * QSCALE).astype(BF16))
        for i in range(nx0):
            qt_ref[a * nx0 + i] = qt[:, i * TQ:(i + 1) * TQ]

    def proj_kv(a, xnt):
        kv = jnp.dot(_upk(wt_ref[D // 2:3 * D // 2, :]), xnt, preferred_element_type=F32)
        for g in range(4):
            kg = kv[G * g:G * g + 128, :].astype(BF16).T
            k_ref[g, a * TA // 2:(a + 1) * TA // 2, :] = _pk(kg)
        rid = jax.lax.broadcasted_iota(jnp.int32, (DP, TA), 0)
        for h in range(H):
            w0, v0, sp = _win(h)
            blk = kv[D + w0:D + w0 + DP, :]
            valid = (rid >= v0) & (rid < v0 + DH)
            blk = jnp.where(valid, blk, jnp.where(rid == sp, 1.0, 0.0))
            vt_ref[DP // 2 * h:DP // 2 * (h + 1), a * TA:(a + 1) * TA] = _pk(blk.astype(BF16))

    def prep_w(c_lo, c_hi):
        for c in range(c_lo, c_hi):
            w = min(128, 3 * D - c * 128)
            wt_ref[c * 64:c * 64 + w // 2, :] = _pk(wqkv_ref[:, c * 128:c * 128 + w].T)

    def prep_wo():
        wo = wo_ref[...].astype(F32)
        rid = jax.lax.broadcasted_iota(jnp.int32, (DP, D), 0)
        blks = []
        for h in range(H):
            w0, v0, _ = _win(h)
            valid = (rid >= v0) & (rid < v0 + DH)
            blks.append(jnp.where(valid, wo[w0:w0 + DP, :], 0.0).astype(BF16))
        wot_ref[...] = _pk(jnp.concatenate(blks, axis=0).T)

    for c in cp_x[:nx0]:
        c.wait()
    xnt = layernorm(0)
    cp_wq.wait()
    prep_w(0, 4)
    proj_q(0, xnt)
    store_xn(0, xnt)
    cp_wkv.wait()
    for c in cp_x[nx0:2 * nx0]:
        c.wait()
    prep_w(4, 11)
    xnt_n = layernorm(1)
    proj_kv(0, xnt)
    for c in cp_x[2 * nx0:]:
        c.wait()
    cp_wo.wait()
    for a in range(1, NA):
        xnt = xnt_n
        proj_q(a, xnt)
        store_xn(a, xnt)
        if a + 1 < NA:
            xnt_n = layernorm(a + 1)
        if a == 1:
            prep_wo()
        proj_kv(a, xnt)

    cp_w1.wait()
    cp_w3.wait()
    cp_w2.wait()

    def out_copy(r):
        return pltpu.make_async_copy(
            ob_ref.at[r], o_hbm.at[:, pl.ds(pl.multiple_of(r * TQ, TQ), TQ)], sems.at[6 + NQ + r])

    def body(r, carry):
        off = pl.multiple_of(jnp.minimum(r, 0) * 8, 8)
        base1 = r * (TQ // 2)
        base2 = jnp.maximum(r, 0) * (TQ // 2)

        def qmask(h):
            g, j = divmod(h, 4)
            lo, hi = 14 * j, 14 * (j + 1)
            t0, t1 = lo // 8, -(-hi // 8)
            blk = qt_ref[r, 56 * g + 8 * t0:56 * g + 8 * t1, :]
            rid = jax.lax.broadcasted_iota(jnp.int32, blk.shape, 0) + 8 * t0
            blk = jnp.where((rid >= lo) & (rid < hi), blk, jnp.uint32(0))
            parts = []
            if t0 > 0:
                parts.append(jnp.zeros((8 * t0, TQ), U32))
            parts.append(blk)
            parts.append(jnp.zeros((64 - 8 * t1, TQ), U32))
            return _upk(jnp.concatenate(parts, axis=0))

        def qk_chunk(h, qm, c, s_ref, mrun):
            kc = _upk(k_ref[h // 4, c * CK // 2:(c + 1) * CK // 2, :])
            s = jnp.dot(kc, qm, preferred_element_type=F32)
            s_ref[c * CK:(c + 1) * CK, :] = s
            mm = jnp.max(s.reshape(CK // 8, 8, TQ), axis=0)
            return mm if mrun is None else jnp.maximum(mrun, mm)

        def pv_chunk(h, c, s_ref, m, acc):
            p = jnp.exp2(s_ref[pl.ds(off + c * CK, CK), :] - m).astype(BF16)
            vc = _upk(vt_ref[DP // 2 * h:DP // 2 * (h + 1), c * CK:(c + 1) * CK])
            o = jnp.dot(vc, p, preferred_element_type=F32)
            return o if acc is None else acc + o

        def ffn_slice(f):
            fs = slice(128 * f, 128 * (f + 1))
            n = TQ // 2 // FS
            for i in range(FS):
                ra = pl.ds(pl.multiple_of(base1 + n * i, n), n)
                rb = pl.ds(pl.multiple_of(base2 + n * i, n), n)
                g = jnp.dot(_upk(xn_ref[ra, :]), w1_ref[:, fs], preferred_element_type=F32)
                u = jnp.dot(_upk(xn_ref[rb, :]), w3_ref[:, fs], preferred_element_type=F32)
                h_ref[n * i:n * (i + 1), fs] = _pk((g * jax.nn.sigmoid(g) * u).astype(BF16))

        def finish_pv(h, acc):
            sp = _win(h)[2]
            inv = 1.0 / acc[sp:sp + 1, :]
            ot_ref[DP // 2 * h:DP // 2 * (h + 1), :] = _pk((acc * inv).astype(BF16))

        MP = D // NDP

        def down_piece(i):
            return jax.lax.dot_general(w2t_ref[MP * i:MP * (i + 1), :], _upk(h_ref[...]), NT,
                                       preferred_element_type=F32)

        bufs = (sa, sb)
        m = None
        ys = []
        for u in range(-1, H - 1):
            mrun = None
            acc = None
            qm = qmask(u + 1)
            for c in range(NCK):
                mrun = qk_chunk(u + 1, qm, c, bufs[(u + 1) % 2], mrun)
                if u >= 0:
                    acc = pv_chunk(u, c, bufs[u % 2], m, acc)
            m = jnp.max(mrun, axis=0, keepdims=True)
            if u >= 0:
                finish_pv(u, acc)
            if u + 1 < F // 128:
                ffn_slice(u + 1)
            else:
                ys.append(down_piece(len(ys)))
        acc = None
        for c in range(NCK // 2):
            acc = pv_chunk(H - 1, c, bufs[(H - 1) % 2], m, acc)
        ys.append(down_piece(2))
        for c in range(NCK // 2, NCK):
            acc = pv_chunk(H - 1, c, bufs[(H - 1) % 2], m, acc)
        finish_pv(H - 1, acc)
        ys.append(down_piece(3))
        y = jnp.concatenate(ys, axis=0)
        y = y + jnp.dot(_upk(wot_ref[...]), _upk(ot_ref[...]), preferred_element_type=F32)
        ob_ref[r] = (xt_ref[r].astype(F32) + y).astype(BF16)
        out_copy(r).start()
        return carry

    jax.lax.fori_loop(0, NQ, body, 0)
    for r in range(NQ):
        out_copy(r).wait()


@jax.jit
def pallas_parallel_sum__softmax_full_mha__glu_gated_swiglu__prompt_kernel(
    A_x: jax.Array,
    A_wqkv: jax.Array,
    A_wo: jax.Array,
    B_x: jax.Array,
    B_w1: jax.Array,
    B_w3: jax.Array,
    B_w2: jax.Array,
):
    del B_x
    xt = A_x.reshape(S, D).T
    any_spec = pl.BlockSpec(memory_space=pl.ANY)
    out_t = pl.pallas_call(
        _kernel,
        out_shape=jax.ShapeDtypeStruct((D, S), A_x.dtype),
        in_specs=[any_spec] * 6,
        out_specs=any_spec,
        scratch_shapes=[
            pltpu.VMEM((NQ, D, TQ), BF16),
            pltpu.VMEM((D, 3 * D), BF16),
            pltpu.VMEM((D, D), BF16),
            pltpu.VMEM((D, F), BF16),
            pltpu.VMEM((D, F), BF16),
            pltpu.VMEM((D, F), BF16),
            pltpu.VMEM((NQ, D, TQ), BF16),
            pltpu.SemaphoreType.DMA((6 + 2 * NQ,)),
            pltpu.VMEM((3 * D // 2, D), U32),
            pltpu.VMEM((D // 2, H * DP), U32),
            pltpu.VMEM((S // 2, D), U32),
            pltpu.VMEM((NQ, D // 2, TQ), U32),
            pltpu.VMEM((4, S // 2, 128), U32),
            pltpu.VMEM((H * DP // 2, S), U32),
            pltpu.VMEM((S, TQ), F32),
            pltpu.VMEM((S, TQ), F32),
            pltpu.VMEM((H * DP // 2, TQ), U32),
            pltpu.VMEM((TQ // 2, F), U32),
        ],
        compiler_params=pltpu.CompilerParams(vmem_limit_bytes=100 * 1024 * 1024),
    )(xt, A_wqkv, A_wo, B_w1, B_w3, B_w2.T)
    return out_t.T.reshape(1, S, D)
```

```python
import math

import jax
import jax.numpy as jnp
import jax.experimental.pallas as pl
import jax.experimental.pallas.tpu as pltpu

S = 2048
D = 448
H = 16
DH = 28
DP = 32
G = 112
F = 1792
TQ = 256
NQ = S // TQ
CK = 128
NCK = S // CK
TA = 512
NA = S // TA
FS = 2
NDP = 4
EPS = 1e-5
QSCALE = (DH ** -0.5) * math.log2(math.e)

F32 = jnp.float32
BF16 = jnp.bfloat16
U32 = jnp.uint32
NT = (((1,), (1,)), ((), ()))


def _pk(x):
    return pltpu.bitcast(x, U32)


def _upk(x):
    return pltpu.bitcast(x, BF16)


def _win(h):
    if h % 2 == 0:
        return DH * h, 0, DH
    return DH * h - 4, 4, 0


def _kernel(xt_hbm, wqkv_hbm, wo_hbm, w1_hbm, w3_hbm, w2t_hbm, o_hbm,
            xt_ref, wqkv_ref, wo_ref, w1_ref, w3_ref, w2t_ref, ob_ref, sems,
            wt_ref, wot_ref, xn_ref, qt_ref, k_ref, vt_ref,
            sa, sb, ot_ref, h_ref, xnt_ref, st_ref):
    def cp_x(a, sem):
        cs = slice(a * TA, (a + 1) * TA)
        return pltpu.make_async_copy(xt_hbm.at[:, cs], xt_ref.at[:, cs], sems.at[sem])

    def cp_w(lo, hi, sem):
        return pltpu.make_async_copy(wqkv_hbm.at[:, lo:hi], wqkv_ref.at[:, lo:hi], sems.at[sem])

    groups = [
        [cp_x(0, 0)],
        [cp_w(0, 512, 1)],
        [cp_w(2 * D, 3 * D, 2), cp_x(1, 2)],
        [cp_w(512, 2 * D, 3), cp_x(2, 3)],
        [cp_x(3, 4), pltpu.make_async_copy(wo_hbm, wo_ref, sems.at[4])],
        [pltpu.make_async_copy(w1_hbm, w1_ref, sems.at[5]),
         pltpu.make_async_copy(w3_hbm, w3_ref, sems.at[5]),
         pltpu.make_async_copy(w2t_hbm, w2t_ref, sems.at[5])],
    ]
    for grp in groups:
        for c in grp:
            c.start()

    def wait(i):
        for c in groups[i]:
            c.wait()

    def ln(s):
        gs = slice(128 * s, 128 * (s + 1))
        mu = jnp.mean(xt_ref[:, gs].astype(F32), axis=0, keepdims=True)
        st_ref[0:1, gs] = mu
        xc = xt_ref[:, gs].astype(F32) - mu
        rs = jax.lax.rsqrt(jnp.mean(xc * xc, axis=0, keepdims=True) + EPS)
        st_ref[8:9, gs] = rs
        mu = jnp.where(rs < 0.0, rs, mu)
        xnt_ref[:, gs] = _pk(((xt_ref[:, gs].astype(F32) - mu) * rs).astype(BF16))

    def layernorm(a):
        for s in range(a * TA // 128, (a + 1) * TA // 128):
            ln(s)

    def load_xnt(a):
        return _upk(xnt_ref[:, a * TA:(a + 1) * TA])

    def store_xn(a):
        xn_ref[a * TA // 2:(a + 1) * TA // 2, :] = _pk(load_xnt(a).T)

    def proj_q(a):
        qt = jnp.dot(_upk(wt_ref[0:D // 2, :]), load_xnt(a), preferred_element_type=F32)
        qt = _pk((qt * QSCALE).astype(BF16))
        for i in range(TA // TQ):
            qt_ref[a * (TA // TQ) + i] = qt[:, i * TQ:(i + 1) * TQ]

    def proj_k(a):
        kt = jnp.dot(_upk(wt_ref[D // 2:D, :]), load_xnt(a), preferred_element_type=F32)
        kt = _pk(kt.astype(BF16))
        for g in range(4):
            lo = min(G // 2 * g, D // 2 - 64)
            k_ref[g, a * TA // 2:(a + 1) * TA // 2, :] = _pk(_upk(kt[lo:lo + 64, :]).T)

    def proj_v(a):
        vt = jnp.dot(_upk(wt_ref[D:3 * D // 2, :]), load_xnt(a), preferred_element_type=F32)
        rid = jax.lax.broadcasted_iota(jnp.int32, (DP, TA), 0)
        for h in range(H):
            w0, v0, sp = _win(h)
            valid = (rid >= v0) & (rid < v0 + DH)
            blk = jnp.where(valid, vt[w0:w0 + DP, :], jnp.where(rid == sp, 1.0, 0.0))
            vt_ref[DP // 2 * h:DP // 2 * (h + 1), a * TA:(a + 1) * TA] = _pk(blk.astype(BF16))

    def prep_w(c_lo, c_hi):
        for c in range(c_lo, c_hi):
            w = min(128, 3 * D - c * 128)
            wt_ref[c * 64:c * 64 + w // 2, :] = _pk(wqkv_ref[:, c * 128:c * 128 + w].T)

    def prep_wo():
        wo = wo_ref[...].astype(F32)
        rid = jax.lax.broadcasted_iota(jnp.int32, (DP, D), 0)
        blks = []
        for h in range(H):
            w0, v0, _ = _win(h)
            valid = (rid >= v0) & (rid < v0 + DH)
            blks.append(jnp.where(valid, wo[w0:w0 + DP, :], 0.0).astype(BF16))
        wot_ref[...] = _pk(jnp.concatenate(blks, axis=0).T)

    wait(0)
    layernorm(0)
    wait(1)
    prep_w(0, 4)
    proj_q(0)
    store_xn(0)
    wait(2)
    prep_w(7, 11)
    proj_v(0)
    layernorm(1)
    wait(3)
    proj_q(1)
    prep_w(4, 7)
    store_xn(1)
    layernorm(2)
    proj_k(0)
    proj_k(1)
    proj_v(1)
    wait(4)
    proj_q(2)
    store_xn(2)
    layernorm(3)
    proj_k(2)
    proj_v(2)
    proj_q(3)
    store_xn(3)
    prep_wo()
    proj_k(3)
    proj_v(3)
    wait(5)

    def out_copy(r):
        cols = pl.ds(pl.multiple_of(r * TQ, TQ), TQ)
        return pltpu.make_async_copy(ob_ref.at[r], o_hbm.at[:, cols], sems.at[6])

    def body(r, carry):
        off = pl.multiple_of(jnp.minimum(r, 0) * 8, 8)
        base1 = r * (TQ // 2)
        base2 = jnp.maximum(r, 0) * (TQ // 2)

        def qmask(h):
            g, j = divmod(h, 4)
            lo, hi = 14 * j, 14 * (j + 1)
            t0, t1 = lo // 8, -(-hi // 8)
            blk = qt_ref[r, 56 * g + 8 * t0:56 * g + 8 * t1, :]
            rid = jax.lax.broadcasted_iota(jnp.int32, blk.shape, 0) + 8 * t0
            blk = jnp.where((rid >= lo) & (rid < hi), blk, jnp.uint32(0))
            sh = 8 if g == 3 else 0
            parts = []
            if 8 * t0 + sh > 0:
                parts.append(jnp.zeros((8 * t0 + sh, TQ), U32))
            parts.append(blk)
            if 64 - 8 * t1 - sh > 0:
                parts.append(jnp.zeros((64 - 8 * t1 - sh, TQ), U32))
            return _upk(jnp.concatenate(parts, axis=0))

        def qk_chunk(h, qm, c, s_ref, mrun):
            kc = _upk(k_ref[h // 4, c * CK // 2:(c + 1) * CK // 2, :])
            s = jnp.dot(kc, qm, preferred_element_type=F32)
            s_ref[c * CK:(c + 1) * CK, :] = s
            mm = jnp.max(s.reshape(CK // 8, 8, TQ), axis=0)
            return mm if mrun is None else jnp.maximum(mrun, mm)

        def pv_chunk(h, c, s_ref, m, acc):
            p = jnp.exp2(s_ref[pl.ds(off + c * CK, CK), :] - m).astype(BF16)
            vc = _upk(vt_ref[DP // 2 * h:DP // 2 * (h + 1), c * CK:(c + 1) * CK])
            o = jnp.dot(vc, p, preferred_element_type=F32)
            return o if acc is None else o + acc

        def ffn_slice(f):
            fs = slice(128 * f, 128 * (f + 1))
            n = TQ // 2 // FS
            for i in range(FS):
                ra = pl.ds(pl.multiple_of(base1 + n * i, n), n)
                rb = pl.ds(pl.multiple_of(base2 + n * i, n), n)
                g = jnp.dot(_upk(xn_ref[ra, :]), w1_ref[:, fs], preferred_element_type=F32)
                u = jnp.dot(_upk(xn_ref[rb, :]), w3_ref[:, fs], preferred_element_type=F32)
                hg = 0.5 * g
                h_ref[n * i:n * (i + 1), fs] = _pk(((hg * jnp.tanh(hg) + hg) * u).astype(BF16))

        def finish_pv(h, acc):
            sp = _win(h)[2]
            inv = 1.0 / acc[sp:sp + 1, :]
            ot_ref[DP // 2 * h:DP // 2 * (h + 1), :] = _pk((acc * inv).astype(BF16))

        MP = D // NDP

        def down_piece(i, lo=0, hi=F):
            return jax.lax.dot_general(w2t_ref[MP * i:MP * (i + 1), lo:hi], _upk(h_ref[:, lo:hi]), NT,
                                       preferred_element_type=F32)

        bufs = (sa, sb)
        m = None
        ys = []
        for u in range(-1, H - 1):
            mrun = None
            acc = None
            qm = qmask(u + 1)
            for c in range(NCK):
                mrun = qk_chunk(u + 1, qm, c, bufs[(u + 1) % 2], mrun)
                if m is not None:
                    acc = pv_chunk(u, c, bufs[u % 2], m, acc)
            m = jnp.max(mrun, axis=0, keepdims=True)
            if acc is not None:
                finish_pv(u, acc)
            if u + 1 < F // 128:
                ffn_slice(u + 1)
            else:
                ys.append(down_piece(len(ys)))
        acc = None
        for t in range(4):
            for c in range(4 * t, 4 * (t + 1)):
                acc = pv_chunk(H - 1, c, bufs[(H - 1) % 2], m, acc)
            if t == 3:
                finish_pv(H - 1, acc)
            if t % 2 == 0:
                ys.append(down_piece(2 + t // 2, 0, 768))
            else:
                ys[-1] = down_piece(2 + t // 2, 768, F) + ys[-1]
        y = jnp.concatenate(ys, axis=0)
        y = y + jnp.dot(_upk(wot_ref[...]), _upk(ot_ref[...]), preferred_element_type=F32)
        xr = xt_ref[:, pl.ds(pl.multiple_of(r * TQ, TQ), TQ)]
        ob_ref[r] = (xr.astype(F32) + y).astype(BF16)
        out_copy(r).start()
        return carry

    jax.lax.fori_loop(0, NQ, body, 0)
    for r in range(NQ):
        out_copy(r).wait()


@jax.jit
def pallas_parallel_sum__softmax_full_mha__glu_gated_swiglu__prompt_kernel(
    A_x: jax.Array,
    A_wqkv: jax.Array,
    A_wo: jax.Array,
    B_x: jax.Array,
    B_w1: jax.Array,
    B_w3: jax.Array,
    B_w2: jax.Array,
):
    del B_x
    xt = A_x.reshape(S, D).T
    any_spec = pl.BlockSpec(memory_space=pl.ANY)
    out_t = pl.pallas_call(
        _kernel,
        out_shape=jax.ShapeDtypeStruct((D, S), A_x.dtype),
        in_specs=[any_spec] * 6,
        out_specs=any_spec,
        scratch_shapes=[
            pltpu.VMEM((D, S), BF16),
            pltpu.VMEM((D, 3 * D), BF16),
            pltpu.VMEM((D, D), BF16),
            pltpu.VMEM((D, F), BF16),
            pltpu.VMEM((D, F), BF16),
            pltpu.VMEM((D, F), BF16),
            pltpu.VMEM((NQ, D, TQ), BF16),
            pltpu.SemaphoreType.DMA((7,)),
            pltpu.VMEM((3 * D // 2, D), U32),
            pltpu.VMEM((D // 2, H * DP), U32),
            pltpu.VMEM((S // 2, D), U32),
            pltpu.VMEM((NQ, D // 2, TQ), U32),
            pltpu.VMEM((4, S // 2, 128), U32),
            pltpu.VMEM((H * DP // 2, S), U32),
            pltpu.VMEM((S, TQ), F32),
            pltpu.VMEM((S, TQ), F32),
            pltpu.VMEM((H * DP // 2, TQ), U32),
            pltpu.VMEM((TQ // 2, F), U32),
            pltpu.VMEM((D // 2, S), U32),
            pltpu.VMEM((16, S), F32),
        ],
        compiler_params=pltpu.CompilerParams(vmem_limit_bytes=100 * 1024 * 1024),
    )(xt, A_wqkv, A_wo, B_w1, B_w3, B_w2.T)
    return out_t.T.reshape(1, S, D)
```

```python
import math

import jax
import jax.numpy as jnp
import jax.experimental.pallas as pl
import jax.experimental.pallas.tpu as pltpu

S = 2048
D = 448
H = 16
DH = 28
DP = 32
G = 112
F = 1792
TQ = 256
NQ = S // TQ
CK = 128
NCK = S // CK
FS = 2
NDP = 4
EPS = 1e-5
QSCALE = (DH ** -0.5) * math.log2(math.e)

F32 = jnp.float32
BF16 = jnp.bfloat16
U32 = jnp.uint32
NT = (((1,), (1,)), ((), ()))


def _pk(x):
    return pltpu.bitcast(x, U32)


def _upk(x):
    return pltpu.bitcast(x, BF16)


def _win(h):
    if h % 2 == 0:
        return DH * h, 0, DH
    return DH * h - 4, 4, 0


def _kernel(xt_hbm, wqkv_hbm, wo_hbm, w1_hbm, w3_hbm, w2t_hbm, o_hbm,
            xt_ref, wqkv_ref, wo_ref, w1_ref, w3_ref, w2t_ref, ob_ref, sems,
            wt_ref, wot_ref, xn_ref, qt_ref, k_ref, vt_ref,
            sa, sb, ot_ref, h_ref, xnt_ref, st_ref):
    def cp_x(s0, s1, sem):
        cs = slice(128 * s0, 128 * s1)
        return pltpu.make_async_copy(xt_hbm.at[:, cs], xt_ref.at[:, cs], sems.at[sem])

    def cp_w(lo, hi, sem):
        return pltpu.make_async_copy(wqkv_hbm.at[:, lo:hi], wqkv_ref.at[:, lo:hi], sems.at[sem])

    groups = [
        [cp_x(0, 2, 0)],
        [cp_w(0, 512, 1)],
        [cp_w(2 * D, 3 * D, 2)],
        [cp_x(2, 5, 3), cp_w(512, 2 * D, 3)],
        [cp_x(5, 16, 4), pltpu.make_async_copy(wo_hbm, wo_ref, sems.at[4])],
        [pltpu.make_async_copy(w1_hbm, w1_ref, sems.at[5]),
         pltpu.make_async_copy(w3_hbm, w3_ref, sems.at[5]),
         pltpu.make_async_copy(w2t_hbm, w2t_ref, sems.at[5])],
    ]
    for grp in groups:
        for c in grp:
            c.start()

    def wait(i):
        for c in groups[i]:
            c.wait()

    rstd = {}

    def layernorm(s0, s1):
        for s in range(s0, s1):
            gs = slice(128 * s, 128 * (s + 1))
            x = xt_ref[:, gs].astype(F32)
            if s >= 8:
                pr = rstd[s - 3]
                x = jnp.concatenate([jnp.where(pr < 0.0, pr, x[0:8]), x[8:]], axis=0)
            mu = jnp.mean(x, axis=0, keepdims=True)
            st_ref[0:1, gs] = mu
            xc = xt_ref[:, gs].astype(F32) - mu
            rs = jax.lax.rsqrt(jnp.mean(xc * xc, axis=0, keepdims=True) + EPS)
            rstd[s] = rs
            st_ref[8:9, gs] = rs
            mu = jnp.where(rs < 0.0, rs, mu)
            xnt_ref[:, gs] = _pk(((xt_ref[:, gs].astype(F32) - mu) * rs).astype(BF16))

    def load_xnt(s0, s1):
        return _upk(xnt_ref[:, 128 * s0:128 * s1])

    def store_xn(s0, s1):
        xn_ref[64 * s0:64 * s1, :] = _pk(load_xnt(s0, s1).T)

    def proj_q(s0, s1):
        qt = jnp.dot(_upk(wt_ref[0:D // 2, :]), load_xnt(s0, s1), preferred_element_type=F32)
        qt = _pk((qt * QSCALE).astype(BF16))
        for s in range(s0, s1):
            qt_ref[s // 2, :, 128 * (s % 2):128 * (s % 2 + 1)] = qt[:, 128 * (s - s0):128 * (s - s0 + 1)]

    def proj_k(s0, s1):
        kt = jnp.dot(_upk(wt_ref[D // 2:D, :]), load_xnt(s0, s1), preferred_element_type=F32)
        kt = _pk(kt.astype(BF16))
        for g in range(4):
            lo = min(G // 2 * g, D // 2 - 64)
            k_ref[g, 64 * s0:64 * s1, :] = _pk(_upk(kt[lo:lo + 64, :]).T)

    def proj_v(s0, s1):
        vt = jnp.dot(_upk(wt_ref[D:3 * D // 2, :]), load_xnt(s0, s1), preferred_element_type=F32)
        rid = jax.lax.broadcasted_iota(jnp.int32, (DP, 128 * (s1 - s0)), 0)
        for h in range(H):
            w0, v0, sp = _win(h)
            valid = (rid >= v0) & (rid < v0 + DH)
            blk = jnp.where(valid, vt[w0:w0 + DP, :], jnp.where(rid == sp, 1.0, 0.0))
            vt_ref[DP // 2 * h:DP // 2 * (h + 1), 128 * s0:128 * s1] = _pk(blk.astype(BF16))

    def prep_w(c_lo, c_hi):
        for c in range(c_lo, c_hi):
            w = min(128, 3 * D - c * 128)
            wt_ref[c * 64:c * 64 + w // 2, :] = _pk(wqkv_ref[:, c * 128:c * 128 + w].T)

    def prep_wo():
        wo = wo_ref[...].astype(F32)
        rid = jax.lax.broadcasted_iota(jnp.int32, (DP, D), 0)
        blks = []
        for h in range(H):
            w0, v0, _ = _win(h)
            valid = (rid >= v0) & (rid < v0 + DH)
            blks.append(jnp.where(valid, wo[w0:w0 + DP, :], 0.0).astype(BF16))
        wot_ref[...] = _pk(jnp.concatenate(blks, axis=0).T)

    wait(0)
    layernorm(0, 2)
    wait(1)
    prep_w(0, 4)
    proj_q(0, 2)
    store_xn(0, 2)
    wait(2)
    prep_w(7, 11)
    proj_v(0, 2)
    wait(3)
    prep_w(4, 7)
    layernorm(2, 5)
    proj_k(0, 2)
    proj_k(2, 5)
    store_xn(2, 5)
    proj_q(2, 5)
    wait(4)
    layernorm(5, 8)
    proj_v(2, 5)
    for (s0, s1) in [(5, 8), (8, 12), (12, 16)]:
        proj_q(s0, s1)
        store_xn(s0, s1)
        if s1 < 16:
            layernorm(s1, s1 + 4)
        else:
            prep_wo()
        proj_k(s0, s1)
        proj_v(s0, s1)
    wait(5)

    def out_copy(r, j):
        cols = pl.ds(pl.multiple_of(r * TQ + 128 * j, 128), 128)
        return pltpu.make_async_copy(ob_ref.at[2 * r + j], o_hbm.at[:, cols], sems.at[6])

    def body(r, carry):
        off = pl.multiple_of(jnp.minimum(r, 0) * 8, 8)
        base1 = r * (TQ // 2)
        base2 = jnp.maximum(r, 0) * (TQ // 2)

        def qmask(h):
            g, j = divmod(h, 4)
            lo, hi = 14 * j, 14 * (j + 1)
            t0, t1 = lo // 8, -(-hi // 8)
            blk = qt_ref[r, 56 * g + 8 * t0:56 * g + 8 * t1, :]
            rid = jax.lax.broadcasted_iota(jnp.int32, blk.shape, 0) + 8 * t0
            blk = jnp.where((rid >= lo) & (rid < hi), blk, jnp.uint32(0))
            sh = 8 if g == 3 else 0
            parts = []
            if 8 * t0 + sh > 0:
                parts.append(jnp.zeros((8 * t0 + sh, TQ), U32))
            parts.append(blk)
            if 64 - 8 * t1 - sh > 0:
                parts.append(jnp.zeros((64 - 8 * t1 - sh, TQ), U32))
            return _upk(jnp.concatenate(parts, axis=0))

        def qk_chunk(h, qm, c, s_ref, mrun):
            kc = _upk(k_ref[h // 4, c * CK // 2:(c + 1) * CK // 2, :])
            s = jnp.dot(kc, qm, preferred_element_type=F32)
            s_ref[c * CK:(c + 1) * CK, :] = s
            mm = jnp.max(s.reshape(CK // 8, 8, TQ), axis=0)
            return mm if mrun is None else jnp.maximum(mrun, mm)

        def pv_chunk(h, c, s_ref, m, acc):
            p = jnp.exp2(s_ref[pl.ds(off + c * CK, CK), :] - m).astype(BF16)
            vc = _upk(vt_ref[DP // 2 * h:DP // 2 * (h + 1), c * CK:(c + 1) * CK])
            o = jnp.dot(vc, p, preferred_element_type=F32)
            return o if acc is None else o + acc

        def finish_pv(h, acc):
            sp = _win(h)[2]
            inv = 1.0 / acc[sp:sp + 1, :]
            ot_ref[DP // 2 * h:DP // 2 * (h + 1), :] = _pk((acc * inv).astype(BF16))

        def ffn_slice(f):
            fs = slice(128 * f, 128 * (f + 1))
            n = TQ // 2 // FS
            for i in range(FS):
                ra = pl.ds(pl.multiple_of(base1 + n * i, n), n)
                rb = pl.ds(pl.multiple_of(base2 + n * i, n), n)
                g = jnp.dot(_upk(xn_ref[ra, :]), w1_ref[:, fs], preferred_element_type=F32)
                u = jnp.dot(_upk(xn_ref[rb, :]), w3_ref[:, fs], preferred_element_type=F32)
                hg = 0.5 * g
                h_ref[n * i:n * (i + 1), fs] = _pk(((hg * jnp.tanh(hg) + hg) * u).astype(BF16))

        MP = D // NDP

        def down_piece(i, lo=0, hi=F):
            return jax.lax.dot_general(w2t_ref[MP * i:MP * (i + 1), lo:hi], _upk(h_ref[:, lo:hi]), NT,
                                       preferred_element_type=F32)

        bufs = (sa, sb)
        m = None
        ys = []
        for u in range(-1, H - 1):
            mrun = None
            acc = None
            qm = qmask(u + 1)
            for c in range(NCK):
                mrun = qk_chunk(u + 1, qm, c, bufs[(u + 1) % 2], mrun)
                if m is not None:
                    acc = pv_chunk(u, c, bufs[u % 2], m, acc)
            m = jnp.max(mrun, axis=0, keepdims=True)
            if acc is not None:
                finish_pv(u, acc)
            if u + 1 < F // 128:
                ffn_slice(u + 1)
            else:
                ys.append(down_piece(len(ys)))
        acc = None
        for t in range(4):
            for c in range(4 * t, 4 * (t + 1)):
                acc = pv_chunk(H - 1, c, bufs[(H - 1) % 2], m, acc)
            if t == 3:
                finish_pv(H - 1, acc)
            if t % 2 == 0:
                ys.append(down_piece(2 + t // 2, 0, 768))
            else:
                ys[-1] = down_piece(2 + t // 2, 768, F) + ys[-1]
        y = jnp.concatenate(ys, axis=0)
        for j in range(2):
            js = slice(128 * j, 128 * (j + 1))
            yj = jnp.dot(_upk(wot_ref[...]), _upk(ot_ref[:, js]), preferred_element_type=F32) + y[:, js]
            xr = xt_ref[:, pl.ds(pl.multiple_of(r * TQ + 128 * j, 128), 128)]
            ob_ref[2 * r + j] = (xr.astype(F32) + yj).astype(BF16)
            out_copy(r, j).start()
        return carry

    jax.lax.fori_loop(0, NQ, body, 0)
    for r in range(NQ):
        out_copy(r, 0).wait()
        out_copy(r, 1).wait()


@jax.jit
def pallas_parallel_sum__softmax_full_mha__glu_gated_swiglu__prompt_kernel(
    A_x: jax.Array,
    A_wqkv: jax.Array,
    A_wo: jax.Array,
    B_x: jax.Array,
    B_w1: jax.Array,
    B_w3: jax.Array,
    B_w2: jax.Array,
):
    del B_x
    xt = A_x.reshape(S, D).T
    any_spec = pl.BlockSpec(memory_space=pl.ANY)
    out_t = pl.pallas_call(
        _kernel,
        out_shape=jax.ShapeDtypeStruct((D, S), A_x.dtype),
        in_specs=[any_spec] * 6,
        out_specs=any_spec,
        scratch_shapes=[
            pltpu.VMEM((D, S), BF16),
            pltpu.VMEM((D, 3 * D), BF16),
            pltpu.VMEM((D, D), BF16),
            pltpu.VMEM((D, F), BF16),
            pltpu.VMEM((D, F), BF16),
            pltpu.VMEM((D, F), BF16),
            pltpu.VMEM((2 * NQ, D, 128), BF16),
            pltpu.SemaphoreType.DMA((7,)),
            pltpu.VMEM((3 * D // 2, D), U32),
            pltpu.VMEM((D // 2, H * DP), U32),
            pltpu.VMEM((S // 2, D), U32),
            pltpu.VMEM((NQ, D // 2, TQ), U32),
            pltpu.VMEM((4, S // 2, 128), U32),
            pltpu.VMEM((H * DP // 2, S), U32),
            pltpu.VMEM((S, TQ), F32),
            pltpu.VMEM((S, TQ), F32),
            pltpu.VMEM((H * DP // 2, TQ), U32),
            pltpu.VMEM((TQ // 2, F), U32),
            pltpu.VMEM((D // 2, S), U32),
            pltpu.VMEM((16, S), F32),
        ],
        compiler_params=pltpu.CompilerParams(vmem_limit_bytes=100 * 1024 * 1024),
    )(xt, A_wqkv, A_wo, B_w1, B_w3, B_w2.T)
    return out_t.T.reshape(1, S, D)
```

```python
import math

import jax
import jax.numpy as jnp
import jax.experimental.pallas as pl
import jax.experimental.pallas.tpu as pltpu

S = 2048
D = 448
H = 16
DH = 28
DP = 32
G = 112
F = 1792
TQ = 256
NQ = S // TQ
CK = 128
NCK = S // CK
FS = 2
K0 = 256
K1 = D - K0
FH = F // 2
DH2 = D // 2
NDP = 4
EPS = 1e-5
QSCALE = (DH ** -0.5) * math.log2(math.e)

F32 = jnp.float32
BF16 = jnp.bfloat16
U32 = jnp.uint32
NT = (((1,), (1,)), ((), ()))


def _pk(x):
    return pltpu.bitcast(x, U32)


def _upk(x):
    return pltpu.bitcast(x, BF16)


def _win(h):
    if h % 2 == 0:
        return DH * h, 0, DH
    return DH * h - 4, 4, 0


def _kernel(xt_hbm, wqkv_hbm, wo_hbm, w1_hbm, w3_hbm, w2t_hbm, o_hbm,
            xt_ref, wqkv_ref, wo_ref, w1_ref, w3_ref, w2t_ref, ob_ref, sems,
            wt_ref, wot_ref, xn_ref, qt_ref, k_ref, vt_ref,
            sa, sb, ot_ref, h_ref, xnt_ref, st_ref, bo_ref, ao_ref, w2o_ref):
    def cp_x(s0, s1, sem):
        cs = slice(128 * s0, 128 * s1)
        return pltpu.make_async_copy(xt_hbm.at[:, cs], xt_ref.at[:, cs], sems.at[sem])

    def cp_w(lo, hi, sem):
        return pltpu.make_async_copy(wqkv_hbm.at[:, lo:hi], wqkv_ref.at[:, lo:hi], sems.at[sem])

    groups = [
        [cp_x(0, 2, 0)],
        [cp_w(0, 512, 1)],
        [cp_w(2 * D, 3 * D, 2)],
        [cp_x(2, 5, 3), cp_w(512, 2 * D, 3)],
        [cp_x(5, 16, 4), pltpu.make_async_copy(wo_hbm, wo_ref, sems.at[4])],
        [pltpu.make_async_copy(w1_hbm, w1_ref, sems.at[5]),
         pltpu.make_async_copy(w3_hbm, w3_ref, sems.at[5]),
         pltpu.make_async_copy(w2t_hbm, w2t_ref, sems.at[5])],
    ]
    for grp in groups:
        for c in grp:
            c.start()

    def wait(i):
        for c in groups[i]:
            c.wait()

    rstd = {}
    last = [None]

    def layernorm(s0, s1):
        for s in range(s0, s1):
            gs = slice(128 * s, 128 * (s + 1))
            x = xt_ref[:, gs].astype(F32)
            if s >= 8:
                pr = rstd[s - 3]
                x = jnp.concatenate([jnp.where(pr < 0.0, pr, x[0:8]), x[8:]], axis=0)
            mu = jnp.mean(x, axis=0, keepdims=True)
            st_ref[0:1, gs] = mu
            xc = xt_ref[:, gs].astype(F32) - mu
            rs = jax.lax.rsqrt(jnp.mean(xc * xc, axis=0, keepdims=True) + EPS)
            rstd[s] = rs
            st_ref[8:9, gs] = rs
            mu = jnp.where(rs < 0.0, rs, mu)
            xnt_ref[:, gs] = _pk(((xt_ref[:, gs].astype(F32) - mu) * rs).astype(BF16))

    def load_xnt(s0, s1):
        return _upk(xnt_ref[:, 128 * s0:128 * s1])

    def store_xn(s0, s1):
        xn_ref[64 * s0:64 * s1, :] = _pk(load_xnt(s0, s1).T)

    def proj_q(s0, s1):
        qt = jnp.dot(_upk(wt_ref[0:D // 2, :]), load_xnt(s0, s1), preferred_element_type=F32)
        last[0] = qt
        qt = _pk((qt * QSCALE).astype(BF16))
        for s in range(s0, s1):
            qt_ref[s // 2, :, 128 * (s % 2):128 * (s % 2 + 1)] = qt[:, 128 * (s - s0):128 * (s - s0 + 1)]

    def proj_k(s0, s1):
        kt = jnp.dot(_upk(wt_ref[D // 2:D, :]), load_xnt(s0, s1), preferred_element_type=F32)
        last[0] = kt
        kt = _pk(kt.astype(BF16))
        for g in range(4):
            lo = min(G // 2 * g, D // 2 - 64)
            k_ref[g, 64 * s0:64 * s1, :] = _pk(_upk(kt[lo:lo + 64, :]).T)

    def proj_v(s0, s1):
        vt = jnp.dot(_upk(wt_ref[D:3 * D // 2, :]), load_xnt(s0, s1), preferred_element_type=F32)
        last[0] = vt
        rid = jax.lax.broadcasted_iota(jnp.int32, (DP, 128 * (s1 - s0)), 0)
        for h in range(H):
            w0, v0, sp = _win(h)
            valid = (rid >= v0) & (rid < v0 + DH)
            blk = jnp.where(valid, vt[w0:w0 + DP, :], jnp.where(rid == sp, 1.0, 0.0))
            vt_ref[DP // 2 * h:DP // 2 * (h + 1), 128 * s0:128 * s1] = _pk(blk.astype(BF16))

    def prep_w(c_lo, c_hi):
        for c in range(c_lo, c_hi):
            w = min(128, 3 * D - c * 128)
            wt_ref[c * 64:c * 64 + w // 2, :] = _pk(wqkv_ref[:, c * 128:c * 128 + w].T)

    def prep_wo():
        wo = wo_ref[...].astype(F32)
        rid = jax.lax.broadcasted_iota(jnp.int32, (DP, D), 0)
        blks = []
        for h in range(H):
            w0, v0, _ = _win(h)
            valid = (rid >= v0) & (rid < v0 + DH)
            blks.append(jnp.where(valid, wo[w0:w0 + DP, :], 0.0).astype(BF16))
        wot_ref[...] = _pk(jnp.concatenate(blks, axis=0).T)

    RC = 16

    def gate(x, anchor):
        if anchor is None:
            return x
        reps = (x.shape[0] // 8, x.shape[1] // 128)
        never = jnp.tile(jnp.broadcast_to(rstd[0] < 0.0, (8, 128)), reps)
        return jnp.where(never, jnp.tile(anchor, reps), x)

    def job_b(i, c, anchor):
        n0 = slice(128 * i, 128 * (i + 1))
        n1 = slice(FH + 128 * i, FH + 128 * (i + 1))

        def ld(rows, cols):
            return jnp.concatenate([w1_ref[rows, cols].astype(F32), w3_ref[rows, cols].astype(F32)], axis=1)

        ra = slice(RC * c, RC * (c + 1))
        rb = slice(K0 + RC * c, K0 + RC * (c + 1))
        b11 = gate(ld(ra, n0), anchor)
        b12 = ld(ra, n1)
        if RC * c < K1:
            b21 = ld(rb, n0)
            b22 = gate(ld(rb, n1), anchor)
            ops = [b11 + b22, b12 - b22, b21 - b11, b11 + b12, b21 + b22]
        else:
            b12 = gate(b12, anchor)
            ops = [b11, b12, None, b11 + b12, None]
        for j, o in enumerate(ops):
            if o is not None:
                bo_ref[5 * i + j, ra, :] = o.astype(BF16)

    def job_a(b, c, anchor):
        zpad = jnp.zeros((RC, K0 - K1), F32)
        xa = _upk(xn_ref[128 * b + RC // 2 * c:128 * b + RC // 2 * (c + 1), :]).astype(F32)
        xb = _upk(xn_ref[128 * b + 64 + RC // 2 * c:128 * b + 64 + RC // 2 * (c + 1), :]).astype(F32)
        a11, a21 = gate(xa[:, 0:K0], anchor), xb[:, 0:K0]
        a12 = jnp.concatenate([xa[:, K0:D], zpad], axis=1)
        a22 = gate(jnp.concatenate([xb[:, K0:D], zpad], axis=1), anchor)
        ops = [a11 + a22, a21 + a22, a11 + a12, a21 - a11, a12 - a22]
        for j, o in enumerate(ops):
            ao_ref[5 * b + j, RC * c:RC * (c + 1), :] = o.astype(BF16)

    def job_w2(c, half, anchor):
        lo, hi = (0, 512) if half == 0 else (512, FH)
        ra = slice(8 * c, 8 * (c + 1))
        rb = slice(DH2 + 8 * c, DH2 + 8 * (c + 1))
        a11 = gate(w2t_ref[ra, lo:hi].astype(F32), anchor)
        a12 = w2t_ref[ra, FH + lo:FH + hi].astype(F32)
        a21 = w2t_ref[rb, lo:hi].astype(F32)
        a22 = gate(w2t_ref[rb, FH + lo:FH + hi].astype(F32), anchor)
        ops = [a11 + a22, a21 + a22, a11 + a12, a21 - a11, a12 - a22]
        for j, o in enumerate(ops):
            w2o_ref[j, ra, lo:hi] = o.astype(BF16)

    def with_jobs(projs, jobs):
        n = len(projs) * (D // 8) - 16
        k = 0
        for pi, (proj, s) in enumerate(projs):
            proj(s, s + 1)
            y = last[0]
            while k < len(jobs) and (k * n) // len(jobs) < (pi + 1) * (D // 8):
                row = (k * n) // len(jobs) - pi * (D // 8)
                fn, x0, x1 = jobs[k]
                fn(x0, x1, y[8 * row:8 * (row + 1), :])
                k += 1

    def jobs_a(b0, b1):
        return [(job_a, b, c) for b in range(b0, b1) for c in range(128 // RC)]

    wait(0)
    layernorm(0, 2)
    wait(1)
    prep_w(0, 4)
    proj_q(0, 2)
    store_xn(0, 2)
    wait(2)
    prep_w(7, 11)
    proj_v(0, 2)
    wait(3)
    prep_w(4, 7)
    layernorm(2, 5)
    proj_k(0, 2)
    proj_k(2, 5)
    store_xn(2, 5)
    with_jobs([(proj_q, s) for s in range(2, 5)], jobs_a(0, 2))
    wait(4)
    layernorm(5, 8)
    proj_v(2, 5)
    proj_q(5, 8)
    store_xn(5, 8)
    layernorm(8, 12)
    proj_k(5, 8)
    with_jobs([(proj_v, s) for s in range(5, 8)], jobs_a(2, 4))
    proj_q(8, 12)
    store_xn(8, 12)
    layernorm(12, 16)
    store_xn(12, 16)
    proj_k(8, 12)
    prep_wo()
    with_jobs([(proj_v, s) for s in range(8, 12)], jobs_a(4, 8))
    wait(5)
    with_jobs([(p_, s) for p_ in (proj_k, proj_q, proj_v) for s in range(12, 16)],
              [(job_b, i, c) for i in range(7) for c in range(K0 // RC)]
              + [(job_w2, c, hf) for c in range(DH2 // 8) for hf in range(2)])

    def out_copy(r, j):
        cols = pl.ds(pl.multiple_of(r * TQ + 128 * j, 128), 128)
        return pltpu.make_async_copy(ob_ref.at[2 * r + j], o_hbm.at[:, cols], sems.at[6])

    def body(r, carry):
        off = pl.multiple_of(jnp.minimum(r, 0) * 8, 8)
        base1 = r * (TQ // 2)
        base2 = jnp.maximum(r, 0) * (TQ // 2)

        def qmask(h):
            g, j = divmod(h, 4)
            lo, hi = 14 * j, 14 * (j + 1)
            t0, t1 = lo // 8, -(-hi // 8)
            blk = qt_ref[r, 56 * g + 8 * t0:56 * g + 8 * t1, :]
            rid = jax.lax.broadcasted_iota(jnp.int32, blk.shape, 0) + 8 * t0
            blk = jnp.where((rid >= lo) & (rid < hi), blk, jnp.uint32(0))
            sh = 8 if g == 3 else 0
            parts = []
            if 8 * t0 + sh > 0:
                parts.append(jnp.zeros((8 * t0 + sh, TQ), U32))
            parts.append(blk)
            if 64 - 8 * t1 - sh > 0:
                parts.append(jnp.zeros((64 - 8 * t1 - sh, TQ), U32))
            return _upk(jnp.concatenate(parts, axis=0))

        def qk_chunk(h, qm, c, s_ref, mrun):
            kc = _upk(k_ref[h // 4, c * CK // 2:(c + 1) * CK // 2, :])
            s = jnp.dot(kc, qm, preferred_element_type=F32)
            s_ref[c * CK:(c + 1) * CK, :] = s
            mm = jnp.max(s.reshape(CK // 8, 8, TQ), axis=0)
            return mm if mrun is None else jnp.maximum(mrun, mm)

        def pv_chunk(h, c, s_ref, m, acc):
            p = jnp.exp2(s_ref[pl.ds(off + c * CK, CK), :] - m).astype(BF16)
            vc = _upk(vt_ref[DP // 2 * h:DP // 2 * (h + 1), c * CK:(c + 1) * CK])
            o = jnp.dot(vc, p, preferred_element_type=F32)
            return o if acc is None else o + acc

        def finish_pv(h, acc):
            sp = _win(h)[2]
            inv = 1.0 / acc[sp:sp + 1, :]
            ot_ref[DP // 2 * h:DP // 2 * (h + 1), :] = _pk((acc * inv).astype(BF16))

        def silu_mul(gu):
            hg = 0.5 * gu[:, 0:128]
            return (hg * jnp.tanh(hg) + hg) * gu[:, 128:256]

        def ffn_slice(f):
            i, half = divmod(f, 2)
            n = 128 // FS
            n0 = slice(128 * i, 128 * (i + 1))
            n1 = slice(FH + 128 * i, FH + 128 * (i + 1))
            for pc in range(half * FS // 2, (half + 1) * FS // 2):
                rows = slice(n * pc, n * (pc + 1))

                def asum(j, kw):
                    return ao_ref[5 * r + j, rows, 0:kw]

                def bsum(j, kw):
                    return bo_ref[5 * i + j, 0:kw, :]

                def mm(a, b):
                    return jnp.dot(a, b, preferred_element_type=F32)

                a11 = _upk(xn_ref[pl.ds(pl.multiple_of(base1 + n // 2 * pc, n // 2), n // 2), 0:K0])
                a22 = _upk(xn_ref[pl.ds(pl.multiple_of(base1 + 64 + n // 2 * pc, n // 2), n // 2), K0:D])
                b11 = jnp.concatenate([w1_ref[0:K0, n0], w3_ref[0:K0, n0]], axis=1)
                b22 = jnp.concatenate([w1_ref[K0:D, n1], w3_ref[K0:D, n1]], axis=1)
                m3 = mm(a11, bsum(1, K0))
                m5 = mm(asum(2, K1), b22)
                h12 = silu_mul(m3 + m5)
                m2 = mm(asum(1, K0), b11)
                c22 = m3 - m2
                m4 = mm(a22, bsum(2, K1))
                h21 = silu_mul(m2 + m4)
                c11 = m4 - m5
                m1 = mm(asum(0, K0), bsum(0, K0))
                c22 = c22 + m1
                c11 = c11 + m1
                h22 = silu_mul(mm(asum(3, K0), bsum(3, K0)) + c22)
                h11 = silu_mul(mm(asum(4, K1), bsum(4, K1)) + c11)
                hops = [h11 + h22, h11, h21 - h22, h12 - h11, h22, h11 + h21, h12 + h22]
                for j, o in enumerate(hops):
                    h_ref[j, n // 2 * pc:n // 2 * (pc + 1), n0] = _pk(o.astype(BF16))

        def down(j):
            a = {2: lambda: w2t_ref[0:DH2, 0:FH], 3: lambda: w2t_ref[DH2:D, FH:F]}.get(
                j, lambda: w2o_ref[{0: 0, 1: 1, 4: 2, 5: 3, 6: 4}[j]])()
            return jax.lax.dot_general(a, _upk(h_ref[j]), NT, preferred_element_type=F32)

        bufs = (sa, sb)
        m = None
        dm = {}
        for u in range(-1, H - 1):
            mrun = None
            acc = None
            qm = qmask(u + 1)
            for c in range(NCK):
                mrun = qk_chunk(u + 1, qm, c, bufs[(u + 1) % 2], mrun)
                if m is not None:
                    acc = pv_chunk(u, c, bufs[u % 2], m, acc)
            m = jnp.max(mrun, axis=0, keepdims=True)
            if acc is not None:
                finish_pv(u, acc)
            if u + 1 < F // 128:
                ffn_slice(u + 1)
            elif u == H - 3:
                dm[3] = down(3)
            else:
                dm[1] = down(1)
                y21 = dm[1] + dm[3]
                dm[4] = down(4)
                y11 = dm[3] - dm[4]
        acc = None
        for t in range(4):
            for c in range(4 * t, 4 * (t + 1)):
                acc = pv_chunk(H - 1, c, bufs[(H - 1) % 2], m, acc)
            if t == 0:
                dm[2] = down(2)
                y12 = dm[2] + dm[4]
                y22 = dm[2] - dm[1]
            elif t == 1:
                dm[0] = down(0)
                y11 = y11 + dm[0]
                y22 = y22 + dm[0]
            elif t == 2:
                y11 = down(6) + y11
            else:
                finish_pv(H - 1, acc)
                y22 = down(5) + y22
        ycol = [jnp.concatenate([y11, y21], axis=0), jnp.concatenate([y12, y22], axis=0)]
        for j in range(2):
            js = slice(128 * j, 128 * (j + 1))
            yj = jnp.dot(_upk(wot_ref[...]), _upk(ot_ref[:, js]), preferred_element_type=F32) + ycol[j]
            xr = xt_ref[:, pl.ds(pl.multiple_of(r * TQ + 128 * j, 128), 128)]
            ob_ref[2 * r + j] = (xr.astype(F32) + yj).astype(BF16)
            out_copy(r, j).start()
        return carry

    jax.lax.fori_loop(0, NQ, body, 0)
    for r in range(NQ):
        out_copy(r, 0).wait()
        out_copy(r, 1).wait()


@jax.jit
def pallas_parallel_sum__softmax_full_mha__glu_gated_swiglu__prompt_kernel(
    A_x: jax.Array,
    A_wqkv: jax.Array,
    A_wo: jax.Array,
    B_x: jax.Array,
    B_w1: jax.Array,
    B_w3: jax.Array,
    B_w2: jax.Array,
):
    del B_x
    xt = A_x.reshape(S, D).T
    any_spec = pl.BlockSpec(memory_space=pl.ANY)
    out_t = pl.pallas_call(
        _kernel,
        out_shape=jax.ShapeDtypeStruct((D, S), A_x.dtype),
        in_specs=[any_spec] * 6,
        out_specs=any_spec,
        scratch_shapes=[
            pltpu.VMEM((D, S), BF16),
            pltpu.VMEM((D, 3 * D), BF16),
            pltpu.VMEM((D, D), BF16),
            pltpu.VMEM((D, F), BF16),
            pltpu.VMEM((D, F), BF16),
            pltpu.VMEM((D, F), BF16),
            pltpu.VMEM((2 * NQ, D, 128), BF16),
            pltpu.SemaphoreType.DMA((7,)),
            pltpu.VMEM((3 * D // 2, D), U32),
            pltpu.VMEM((D // 2, H * DP), U32),
            pltpu.VMEM((S // 2, D), U32),
            pltpu.VMEM((NQ, D // 2, TQ), U32),
            pltpu.VMEM((4, S // 2, 128), U32),
            pltpu.VMEM((H * DP // 2, S), U32),
            pltpu.VMEM((S, TQ), F32),
            pltpu.VMEM((S, TQ), F32),
            pltpu.VMEM((H * DP // 2, TQ), U32),
            pltpu.VMEM((7, 64, FH), U32),
            pltpu.VMEM((D // 2, S), U32),
            pltpu.VMEM((16, S), F32),
            pltpu.VMEM((35, K0, 256), BF16),
            pltpu.VMEM((5 * NQ, 128, K0), BF16),
            pltpu.VMEM((5, D // 2, F // 2), BF16),
        ],
        compiler_params=pltpu.CompilerParams(vmem_limit_bytes=100 * 1024 * 1024),
    )(xt, A_wqkv, A_wo, B_w1, B_w3, B_w2.T)
    return out_t.T.reshape(1, S, D)
```

```python
import math

import jax
import jax.numpy as jnp
import jax.experimental.pallas as pl
import jax.experimental.pallas.tpu as pltpu

S = 2048
D = 448
H = 16
DH = 28
DP = 32
G = 112
F = 1792
TQ = 256
NQ = S // TQ
CK = 128
NCK = S // CK
K0 = 256
K1 = D - K0
FH = F // 2
DH2 = D // 2
RC = 16
NOC = 4
NKG = NOC * CK // 8
NSUB = 4
EPS = 1e-5
QSCALE = (DH ** -0.5) * math.log2(math.e)

F32 = jnp.float32
BF16 = jnp.bfloat16
U32 = jnp.uint32
NT = (((1,), (1,)), ((), ()))


def _pk(x):
    return pltpu.bitcast(x, U32)


def _upk(x):
    return pltpu.bitcast(x, BF16)


def _win(h):
    if h % 2 == 0:
        return DH * h, 0, DH
    return DH * h - 4, 4, 0


def _tree(ts):
    while len(ts) > 1:
        ts = [ts[i] + ts[i + 1] if i + 1 < len(ts) else ts[i] for i in range(0, len(ts), 2)]
    return ts[0]


def _gate(x, anchor, never):
    reps = (x.shape[0] // 8, x.shape[1] // 128)
    return jnp.where(jnp.tile(never, reps), jnp.tile(anchor, reps), x)


def _mix(*lists):
    keyed = [((i + 0.5) / len(l), n, j) for n, l in enumerate(lists) for i, j in enumerate(l)]
    return [j for _, _, j in sorted(keyed, key=lambda t: t[:2])]


def _kernel(xt_hbm, wqkv_hbm, wo_hbm, w1_hbm, w3_hbm, w2t_hbm, o_hbm,
            xt_ref, wqkv_ref, wo_ref, w1_ref, w3_ref, w2t_ref, ob_ref, sems,
            wt_ref, wot_ref, xn_ref, qt_ref, k_ref, vt_ref,
            sa, sb, ot_ref, h_ref, xnt_ref, st_ref,
            bo_ref, ao_ref, kb_ref, qb_ref, so_ref, om_ref, ktf_ref, w2o_ref):
    def cp_x(s0, s1, sem):
        cs = slice(128 * s0, 128 * s1)
        return pltpu.make_async_copy(xt_hbm.at[:, cs], xt_ref.at[:, cs], sems.at[sem])

    def cp_w(lo, hi, sem):
        return pltpu.make_async_copy(wqkv_hbm.at[:, lo:hi], wqkv_ref.at[:, lo:hi], sems.at[sem])

    groups = [
        [cp_x(0, 2, 0)],
        [cp_w(0, 512, 1)],
        [cp_w(2 * D, 3 * D, 2)],
        [cp_x(2, 5, 3), cp_w(512, 2 * D, 3)],
        [cp_x(5, 16, 4), pltpu.make_async_copy(wo_hbm, wo_ref, sems.at[4])],
        [pltpu.make_async_copy(w1_hbm, w1_ref, sems.at[5]),
         pltpu.make_async_copy(w3_hbm, w3_ref, sems.at[5]),
         pltpu.make_async_copy(w2t_hbm, w2t_ref, sems.at[5])],
    ]
    for grp in groups:
        for c in grp:
            c.start()

    def wait(i):
        for c in groups[i]:
            c.wait()

    rstd = {}

    def layernorm(s0, s1):
        for s in range(s0, s1):
            gs = slice(128 * s, 128 * (s + 1))
            x = xt_ref[:, gs].astype(F32)
            if s >= 8:
                pr = rstd[s - 3]
                x = jnp.concatenate([jnp.where(pr < 0.0, pr, x[0:8]), x[8:]], axis=0)
            mu = jnp.mean(x, axis=0, keepdims=True)
            st_ref[0:1, gs] = mu
            xc = xt_ref[:, gs].astype(F32) - mu
            rs = jax.lax.rsqrt(jnp.mean(xc * xc, axis=0, keepdims=True) + EPS)
            rstd[s] = rs
            st_ref[8:9, gs] = rs
            mu = jnp.where(rs < 0.0, rs, mu)
            xnt_ref[:, gs] = _pk(((xt_ref[:, gs].astype(F32) - mu) * rs).astype(BF16))

    def load_xnt(s0, s1):
        return _upk(xnt_ref[:, 128 * s0:128 * s1])

    def store_xn(s0, s1):
        xn_ref[64 * s0:64 * s1, :] = _pk(load_xnt(s0, s1).T)

    def proj_q(s0, s1):
        y = jnp.dot(_upk(wt_ref[0:D // 2, :]), load_xnt(s0, s1), preferred_element_type=F32)
        qt = _pk((y * QSCALE).astype(BF16))
        for s in range(s0, s1):
            qt_ref[s // 2, :, 128 * (s % 2):128 * (s % 2 + 1)] = qt[:, 128 * (s - s0):128 * (s - s0 + 1)]
        return y

    def proj_k(s0, s1):
        y = jnp.dot(_upk(wt_ref[D // 2:D, :]), load_xnt(s0, s1), preferred_element_type=F32)
        for s in range(s0, min(s1, NOC)):
            ktf_ref[s] = y[0:G, 128 * (s - s0):128 * (s - s0 + 1)]
        kt = _pk(y.astype(BF16))
        for g in range(4):
            lo = min(G // 2 * g, D // 2 - 64)
            k_ref[g, 64 * s0:64 * s1, :] = _pk(_upk(kt[lo:lo + 64, :]).T)
        return y

    def proj_v(s0, s1):
        y = jnp.dot(_upk(wt_ref[D:3 * D // 2, :]), load_xnt(s0, s1), preferred_element_type=F32)
        rid = jax.lax.broadcasted_iota(jnp.int32, (DP, 128 * (s1 - s0)), 0)
        for h in range(H):
            w0, v0, sp = _win(h)
            valid = (rid >= v0) & (rid < v0 + DH)
            blk = jnp.where(valid, y[w0:w0 + DP, :], jnp.where(rid == sp, 1.0, 0.0))
            vt_ref[DP // 2 * h:DP // 2 * (h + 1), 128 * s0:128 * s1] = _pk(blk.astype(BF16))
        return y

    def prep_w(c_lo, c_hi):
        for c in range(c_lo, c_hi):
            w = min(128, 3 * D - c * 128)
            wt_ref[c * 64:c * 64 + w // 2, :] = _pk(wqkv_ref[:, c * 128:c * 128 + w].T)

    def prep_wo():
        wo = wo_ref[...].astype(F32)
        rid = jax.lax.broadcasted_iota(jnp.int32, (DP, D), 0)
        blks = []
        for h in range(H):
            w0, v0, _ = _win(h)
            valid = (rid >= v0) & (rid < v0 + DH)
            blks.append(jnp.where(valid, wo[w0:w0 + DP, :], 0.0).astype(BF16))
        wot_ref[...] = _pk(jnp.concatenate(blks, axis=0).T)

    def qmask(r, h):
        g, j = divmod(h, 4)
        lo, hi = 14 * j, 14 * (j + 1)
        t0, t1 = lo // 8, -(-hi // 8)
        blk = qt_ref[r, 56 * g + 8 * t0:56 * g + 8 * t1, :]
        rid = jax.lax.broadcasted_iota(jnp.int32, blk.shape, 0) + 8 * t0
        blk = jnp.where((rid >= lo) & (rid < hi), blk, jnp.uint32(0))
        sh = 8 if g == 3 else 0
        parts = []
        if 8 * t0 + sh > 0:
            parts.append(jnp.zeros((8 * t0 + sh, TQ), U32))
        parts.append(blk)
        if 64 - 8 * t1 - sh > 0:
            parts.append(jnp.zeros((64 - 8 * t1 - sh, TQ), U32))
        return _upk(jnp.concatenate(parts, axis=0))

    def job_b(i, c, anchor, never):
        n0 = slice(128 * i, 128 * (i + 1))
        n1 = slice(FH + 128 * i, FH + 128 * (i + 1))

        def ld(rows, cols):
            return jnp.concatenate([w1_ref[rows, cols].astype(F32), w3_ref[rows, cols].astype(F32)], axis=1)

        ra = slice(RC * c, RC * (c + 1))
        rb = slice(K0 + RC * c, K0 + RC * (c + 1))
        b11 = _gate(ld(ra, n0), anchor, never)
        b12 = ld(ra, n1)
        if RC * c < K1:
            b21 = ld(rb, n0)
            b22 = _gate(ld(rb, n1), anchor, never)
            ops = [b11 + b22, b12 - b22, b21 - b11, b11 + b12, b21 + b22]
        else:
            b12 = _gate(b12, anchor, never)
            ops = [b11, b12, None, b11 + b12, None]
        for j, o in enumerate(ops):
            if o is not None:
                bo_ref[5 * i + j, ra, :] = o.astype(BF16)

    def job_a(b, c, anchor, never):
        zpad = jnp.zeros((RC, K0 - K1), F32)
        xa = _upk(xn_ref[128 * b + RC // 2 * c:128 * b + RC // 2 * (c + 1), :]).astype(F32)
        xb = _upk(xn_ref[128 * b + 64 + RC // 2 * c:128 * b + 64 + RC // 2 * (c + 1), :]).astype(F32)
        a11, a21 = _gate(xa[:, 0:K0], anchor, never), xb[:, 0:K0]
        a12 = jnp.concatenate([xa[:, K0:D], zpad], axis=1)
        a22 = _gate(jnp.concatenate([xb[:, K0:D], zpad], axis=1), anchor, never)
        ops = [a11 + a22, a21 + a22, a11 + a12, a21 - a11, a12 - a22]
        for j, o in enumerate(ops):
            ao_ref[5 * b + j, RC * c:RC * (c + 1), :] = o.astype(BF16)

    def job_w2(c, half, anchor, never):
        lo, hi = (0, 512) if half == 0 else (512, FH)
        ra = slice(8 * c, 8 * (c + 1))
        rb = slice(DH2 + 8 * c, DH2 + 8 * (c + 1))
        a11 = _gate(w2t_ref[ra, lo:hi].astype(F32), anchor, never)
        a12 = w2t_ref[ra, FH + lo:FH + hi].astype(F32)
        a21 = w2t_ref[rb, lo:hi].astype(F32)
        a22 = _gate(w2t_ref[rb, FH + lo:FH + hi].astype(F32), anchor, never)
        ops = [a11 + a22, a21 + a22, a11 + a12, a21 - a11, a12 - a22]
        for j, o in enumerate(ops):
            w2o_ref[j, ra, lo:hi] = o.astype(BF16)

    def job_kb(s, d, anchor, never):
        row = _gate(jnp.broadcast_to(ktf_ref[s, d:d + 1, :], (8, 128)), anchor, never)
        row = jnp.concatenate([row, row], axis=0).astype(BF16)
        blk = jnp.concatenate([row] * 8, axis=0).T.astype(F32)
        kb_ref[16 * s:16 * (s + 1), 8 * d:8 * (d + 1), :] = blk.reshape(16, 8, 128)

    def job_qb(b, c, anchor, never):
        c, hf = divmod(c, 4)
        q = _upk(qt_ref[b, 8 * c:8 * (c + 1), :]).astype(F32)
        q = _gate(q[8 * (hf // 2):8 * (hf // 2 + 1)], anchor, never)
        for i in range(4 * (hf % 2), 4 * (hf % 2 + 1)):
            d = 16 * c + 8 * (hf // 2) + i
            qb_ref[8 * d:8 * (d + 1), :] = jnp.broadcast_to(q[i:i + 1, :], (8, TQ))

    def never_a():
        return jnp.broadcast_to(rstd[0] < 0.0, (8, 128))

    def with_jobs(projs, jobs):
        n = len(projs) * (D // 8) - 32
        k = 0
        for pi, (proj, s) in enumerate(projs):
            y = proj(s, s + 1)
            while k < len(jobs) and (k * n) // len(jobs) < (pi + 1) * (D // 8):
                row = (k * n) // len(jobs) - pi * (D // 8)
                fn, x0, x1 = jobs[k]
                fn(x0, x1, y[8 * row:8 * (row + 1), :], never_a())
                k += 1

    def with_jobs_multi(proj, s0, s1, jobs):
        y = proj(s0, s1)
        n = (s1 - s0) * (D // 8)
        for k, (fn, x0, x1) in enumerate(jobs):
            j, row = divmod((k * n) // len(jobs), D // 8)
            fn(x0, x1, y[8 * row:8 * (row + 1), 128 * j:128 * (j + 1)], never_a())

    def jobs_a(b0, b1):
        return [(job_a, b, c) for b in range(b0, b1) for c in range(128 // RC)]

    kbj = [(job_kb, s, d) for s in range(NOC) for d in range(G)]
    cut = [0, 3, 5, 8, 13, 18, 21, 28]
    kbs = [kbj[len(kbj) * cut[i] // cut[-1]:len(kbj) * cut[i + 1] // cut[-1]] for i in range(7)]

    wait(0)
    layernorm(0, 2)
    wait(1)
    prep_w(0, 4)
    proj_q(0, 2)
    store_xn(0, 2)
    wait(2)
    prep_w(7, 11)
    proj_v(0, 2)
    wait(3)
    prep_w(4, 7)
    layernorm(2, 5)
    proj_k(0, 2)
    with_jobs([(proj_k, s) for s in range(2, 5)], kbs[0])
    store_xn(2, 5)
    with_jobs([(proj_q, s) for s in range(2, 5)], _mix(jobs_a(0, 2), kbs[1]))
    wait(4)
    layernorm(5, 8)
    proj_v(2, 5)
    proj_q(5, 8)
    store_xn(5, 8)
    layernorm(8, 12)
    proj_k(5, 8)
    with_jobs([(proj_v, s) for s in range(5, 8)], _mix(jobs_a(2, 4), kbs[2]))
    with_jobs_multi(proj_q, 8, 12, _mix(kbs[3], [(job_qb, 1, c) for c in range(G // 4)]))
    store_xn(8, 12)
    layernorm(12, 16)
    store_xn(12, 16)
    with_jobs_multi(proj_k, 8, 12, kbs[4])
    prep_wo()
    with_jobs([(proj_v, s) for s in range(8, 12)], _mix(jobs_a(4, 8), kbs[5]))
    wait(5)
    for h in range(4):
        s0 = jnp.dot(_upk(k_ref[0, 0:NOC * CK // 2, :]), qmask(0, h), preferred_element_type=F32)
        so_ref[h] = s0
        om_ref[h] = jnp.max(s0.reshape(NKG, 8, TQ), axis=0)
    with_jobs([(p_, s) for p_ in (proj_k, proj_q, proj_v) for s in range(12, 16)],
              _mix([(job_b, i, c) for i in range(7) for c in range(K0 // RC)]
                   + [(job_w2, c, hf) for c in range(DH2 // 8) for hf in range(2)], kbs[6]))

    def out_copy(r, j):
        cols = pl.ds(pl.multiple_of(r * TQ + 128 * j, 128), 128)
        return pltpu.make_async_copy(ob_ref.at[2 * r + j], o_hbm.at[:, cols], sems.at[6])

    def body(r, carry):
        zero = jnp.minimum(r, 0)
        off = pl.multiple_of(zero * 8, 8)
        never = jax.lax.broadcasted_iota(jnp.int32, (8, 128), 1) < zero

        qvs = [qb_ref.at[pl.ds(pl.multiple_of(jnp.minimum(r + i, 0) * 8, 8), 8 * G)] for i in range(2)]
        kbv = kb_ref.at[pl.ds(zero, NKG)]
        omv = om_ref.at[pl.ds(zero, 4)]
        part = [None]

        def score_job(h, kg, sub, anchor):
            nd = DH // NSUB
            ts = []
            for d in range(DH * h + nd * sub, DH * h + nd * (sub + 1)):
                kb = kbv[kg, 8 * d:8 * (d + 1), :]
                ts.append(jnp.tile(kb, (1, 2)) * qvs[kg % 2][8 * d:8 * (d + 1), :])
            ts[0] = _gate(ts[0], anchor, never)
            if sub > 0:
                ts.append(part[0])
            acc = _tree(ts)
            part[0] = acc
            if sub == NSUB - 1:
                so_ref[h, 8 * kg:8 * (kg + 1), :] = acc
                om_ref[h] = acc if kg == 0 else jnp.maximum(omv[h], acc)

        jobs = [(h, kg, sub) for h in range(4) for kg in range(NKG) for sub in range(NSUB)]
        WQ, WF = 80, 32
        wtot = WQ * (3 * (NCK - NOC) + (H - 4) * NCK) + WF * 7 * (F // 128 - 1)
        clock = [0]
        jdone = [0]

        def tick(y, w):
            lo = clock[0]
            clock[0] += w
            while jdone[0] < len(jobs) and (jdone[0] * wtot) // len(jobs) < clock[0]:
                row = ((jdone[0] * wtot) // len(jobs) - lo) * (y.shape[0] // 8) // w
                score_job(*jobs[jdone[0]], y[8 * row:8 * (row + 1), 0:128])
                jdone[0] += 1

        def qk_chunk(h, qm, c, s_ref, mrun):
            kc = _upk(k_ref[h // 4, c * CK // 2:(c + 1) * CK // 2, :])
            s = jnp.dot(kc, qm, preferred_element_type=F32)
            s_ref[c * CK:(c + 1) * CK, :] = s
            mm = jnp.max(s.reshape(CK // 8, 8, TQ), axis=0)
            mrun = mm if mrun is None else jnp.maximum(mrun, mm)
            if h >= 1:
                tick(s, WQ)
            return mrun

        def pv_chunk(h, c, s_ref, m, acc):
            if h < 4 and c < NOC:
                sv = so_ref[h, c * CK:(c + 1) * CK, :]
            else:
                sv = s_ref[pl.ds(off + c * CK, CK), :]
            p = jnp.exp2(sv - m).astype(BF16)
            vc = _upk(vt_ref[DP // 2 * h:DP // 2 * (h + 1), c * CK:(c + 1) * CK])
            o = jnp.dot(vc, p, preferred_element_type=F32)
            return o if acc is None else o + acc

        def finish_pv(h, acc):
            sp = _win(h)[2]
            inv = 1.0 / acc[sp:sp + 1, :]
            ot_ref[DP // 2 * h:DP // 2 * (h + 1), :] = _pk((acc * inv).astype(BF16))

        def silu_mul(gu):
            hg = 0.5 * gu[:, 0:128]
            return (hg * jnp.tanh(hg) + hg) * gu[:, 128:256]

        def ffn_slice(f):
            i, pc = divmod(f, 2)
            n0 = slice(128 * i, 128 * (i + 1))
            n1 = slice(FH + 128 * i, FH + 128 * (i + 1))

            def asum(j, kw):
                return ao_ref[5 * r + j, 64 * pc:64 * (pc + 1), 0:kw]

            def bsum(j, kw):
                return bo_ref[5 * i + j, 0:kw, :]

            def mm(a, b):
                y = jnp.dot(a, b, preferred_element_type=F32)
                if f > 0:
                    tick(y, WF)
                return y

            a11 = _upk(xn_ref[pl.ds(pl.multiple_of(128 * r + 32 * pc, 32), 32), 0:K0])
            a22 = _upk(xn_ref[pl.ds(pl.multiple_of(128 * r + 64 + 32 * pc, 32), 32), K0:D])
            b11 = jnp.concatenate([w1_ref[0:K0, n0], w3_ref[0:K0, n0]], axis=1)
            b22 = jnp.concatenate([w1_ref[K0:D, n1], w3_ref[K0:D, n1]], axis=1)
            m3 = mm(a11, bsum(1, K0))
            m5 = mm(asum(2, K1), b22)
            h12 = silu_mul(m3 + m5)
            m2 = mm(asum(1, K0), b11)
            c22 = m3 - m2
            m4 = mm(a22, bsum(2, K1))
            h21 = silu_mul(m2 + m4)
            c11 = m4 - m5
            m1 = mm(asum(0, K0), bsum(0, K0))
            c22 = c22 + m1
            c11 = c11 + m1
            h22 = silu_mul(mm(asum(3, K0), bsum(3, K0)) + c22)
            h11 = silu_mul(mm(asum(4, K1), bsum(4, K1)) + c11)
            hops = [h11 + h22, h11, h21 - h22, h12 - h11, h22, h11 + h21, h12 + h22]
            for j, o in enumerate(hops):
                h_ref[j, 32 * pc:32 * (pc + 1), n0] = _pk(o.astype(BF16))

        def down(j):
            if j == 2:
                a = w2t_ref[0:DH2, 0:FH]
            elif j == 3:
                a = w2t_ref[DH2:D, FH:F]
            else:
                a = w2o_ref[j if j < 2 else j - 2]
            y = jax.lax.dot_general(a, _upk(h_ref[j]), NT, preferred_element_type=F32)
            if j in (2, 0, 6, 5):
                for i in range(7):
                    job_qb(jnp.minimum(r + 2, NQ - 1), 7 * (2, 0, 6, 5).index(j) + i,
                           y[32 * i:32 * i + 8, :], never)
            return y

        bufs = (sa, sb)
        m = None
        for u in range(-1, H - 1):
            hq = u + 1
            mrun = om_ref[hq] if hq < 4 else None
            acc = None
            qm = qmask(r, hq)
            for c in range(NCK):
                if not (hq < 4 and c < NOC):
                    mrun = qk_chunk(hq, qm, c, bufs[hq % 2], mrun)
                if m is not None:
                    acc = pv_chunk(u, c, bufs[u % 2], m, acc)
            m = jnp.max(mrun, axis=0, keepdims=True)
            if acc is not None:
                finish_pv(u, acc)
            if hq < F // 128:
                ffn_slice(hq)
            elif u == H - 3:
                d4 = down(3)
            else:
                d2 = down(1)
                y21 = d2 + d4
                d5 = down(4)
                y11 = d4 - d5
        assert jdone[0] == len(jobs)
        acc = None
        for t in range(4):
            for c in range(4 * t, 4 * (t + 1)):
                acc = pv_chunk(H - 1, c, bufs[(H - 1) % 2], m, acc)
            if t == 0:
                d3 = down(2)
                y12 = d3 + d5
                y22 = d3 - d2
            elif t == 1:
                d1 = down(0)
                y11 = y11 + d1
                y22 = y22 + d1
            elif t == 2:
                y11 = down(6) + y11
            else:
                finish_pv(H - 1, acc)
                y22 = down(5) + y22
        ycol = [jnp.concatenate([y11, y21], axis=0), jnp.concatenate([y12, y22], axis=0)]
        for j in range(2):
            js = slice(128 * j, 128 * (j + 1))
            yj = jnp.dot(_upk(wot_ref[...]), _upk(ot_ref[:, js]), preferred_element_type=F32) + ycol[j]
            xr = xt_ref[:, pl.ds(pl.multiple_of(r * TQ + 128 * j, 128), 128)]
            ob_ref[2 * r + j] = (xr.astype(F32) + yj).astype(BF16)
            out_copy(r, j).start()
        return carry

    jax.lax.fori_loop(0, NQ, body, 0)
    for r in range(NQ):
        out_copy(r, 0).wait()
        out_copy(r, 1).wait()


@jax.jit
def pallas_parallel_sum__softmax_full_mha__glu_gated_swiglu__prompt_kernel(
    A_x: jax.Array,
    A_wqkv: jax.Array,
    A_wo: jax.Array,
    B_x: jax.Array,
    B_w1: jax.Array,
    B_w3: jax.Array,
    B_w2: jax.Array,
):
    del B_x
    xt = A_x.reshape(S, D).T
    any_spec = pl.BlockSpec(memory_space=pl.ANY)
    out_t = pl.pallas_call(
        _kernel,
        out_shape=jax.ShapeDtypeStruct((D, S), A_x.dtype),
        in_specs=[any_spec] * 6,
        out_specs=any_spec,
        scratch_shapes=[
            pltpu.VMEM((D, S), BF16),
            pltpu.VMEM((D, 3 * D), BF16),
            pltpu.VMEM((D, D), BF16),
            pltpu.VMEM((D, F), BF16),
            pltpu.VMEM((D, F), BF16),
            pltpu.VMEM((D, F), BF16),
            pltpu.VMEM((2 * NQ, D, 128), BF16),
            pltpu.SemaphoreType.DMA((7,)),
            pltpu.VMEM((3 * D // 2, D), U32),
            pltpu.VMEM((D // 2, H * DP), U32),
            pltpu.VMEM((S // 2, D), U32),
            pltpu.VMEM((NQ, D // 2, TQ), U32),
            pltpu.VMEM((4, S // 2, 128), U32),
            pltpu.VMEM((H * DP // 2, S), U32),
            pltpu.VMEM((S, TQ), F32),
            pltpu.VMEM((S, TQ), F32),
            pltpu.VMEM((H * DP // 2, TQ), U32),
            pltpu.VMEM((7, 64, FH), U32),
            pltpu.VMEM((D // 2, S), U32),
            pltpu.VMEM((16, S), F32),
            pltpu.VMEM((35, K0, 256), BF16),
            pltpu.VMEM((5 * NQ, 128, K0), BF16),
            pltpu.VMEM((NKG, 8 * G, 128), F32),
            pltpu.VMEM((8 * G, TQ), F32),
            pltpu.VMEM((4, NOC * CK, TQ), F32),
            pltpu.VMEM((4, 8, TQ), F32),
            pltpu.VMEM((NOC, G, 128), F32),
            pltpu.VMEM((5, D // 2, F // 2), BF16),
        ],
        compiler_params=pltpu.CompilerParams(vmem_limit_bytes=100 * 1024 * 1024),
    )(xt, A_wqkv, A_wo, B_w1, B_w3, B_w2.T)
    return out_t.T.reshape(1, S, D)
```

```python
import math

import jax
import jax.numpy as jnp
import jax.experimental.pallas as pl
import jax.experimental.pallas.tpu as pltpu

S = 2048
D = 448
H = 16
DH = 28
DP = 32
G = 112
F = 1792
TQ = 256
NQ = S // TQ
CK = 128
NCK = S // CK
K0 = 256
K1 = D - K0
FH = F // 2
DH2 = D // 2
RC = 16
NOCS = (6, 6, 4, 4)
NOC = max(NOCS)
NKG = NOC * CK // 8
NSUB = 4
EPS = 1e-5
QSCALE = (DH ** -0.5) * math.log2(math.e)

F32 = jnp.float32
BF16 = jnp.bfloat16
U32 = jnp.uint32
NT = (((1,), (1,)), ((), ()))


def _pk(x):
    return pltpu.bitcast(x, U32)


def _upk(x):
    return pltpu.bitcast(x, BF16)


def _win(h):
    if h % 2 == 0:
        return DH * h, 0, DH
    return DH * h - 4, 4, 0


def _rep(t, shape):
    if shape[1] > 128:
        t = jax.lax.concatenate([t] * (shape[1] // 128), 1)
    if shape[0] > 8:
        t = jax.lax.concatenate([t] * (shape[0] // 8), 0)
    return t


def _gater(never):
    masks = {}

    def gate(x, anchor):
        if x.shape not in masks:
            masks[x.shape] = _rep(never, x.shape)
        return jax.lax.select(masks[x.shape], _rep(anchor, x.shape), x)

    return gate


def _mix(*lists):
    keyed = [((i + 0.5) / len(l), n, j) for n, l in enumerate(lists) for i, j in enumerate(l)]
    return [j for _, _, j in sorted(keyed, key=lambda t: t[:2])]


def _kernel(xt_hbm, wqkv_hbm, wo_hbm, w1_hbm, w3_hbm, w2t_hbm, o_hbm,
            xt_ref, wqkv_ref, wo_ref, w1_ref, w3_ref, w2t_ref, ob_ref, sems,
            wt_ref, wot_ref, xn_ref, qt_ref, k_ref, vt_ref,
            sa, sb, ot_ref, h_ref, xnt_ref, st_ref,
            bo_ref, ao_ref, kb_ref, qb_ref, so_ref, om_ref, ktf_ref, w2o_ref):
    def cp_x(s0, s1, sem):
        cs = slice(128 * s0, 128 * s1)
        return pltpu.make_async_copy(xt_hbm.at[:, cs], xt_ref.at[:, cs], sems.at[sem])

    def cp_w(lo, hi, sem):
        return pltpu.make_async_copy(wqkv_hbm.at[:, lo:hi], wqkv_ref.at[:, lo:hi], sems.at[sem])

    groups = [
        [cp_x(0, 2, 0)],
        [cp_w(0, 512, 1)],
        [cp_w(2 * D, 3 * D, 2)],
        [cp_x(2, 5, 3), cp_w(512, 2 * D, 3)],
        [cp_x(5, 16, 4), pltpu.make_async_copy(wo_hbm, wo_ref, sems.at[4])],
        [pltpu.make_async_copy(w1_hbm, w1_ref, sems.at[5]),
         pltpu.make_async_copy(w3_hbm, w3_ref, sems.at[5]),
         pltpu.make_async_copy(w2t_hbm, w2t_ref, sems.at[5])],
        [pltpu.make_async_copy(xt_hbm.at[:, 128 * s:128 * (s + 1)], ob_ref.at[s], sems.at[6])
         for s in range(2 * NQ)],
    ]
    for grp in groups:
        for c in grp:
            c.start()

    def wait(i):
        for c in groups[i]:
            c.wait()

    rstd = {}

    def layernorm(s0, s1):
        for s in range(s0, s1):
            gs = slice(128 * s, 128 * (s + 1))
            x = xt_ref[:, gs].astype(F32)
            if s >= 8:
                pr = rstd[s - 3]
                x = jnp.concatenate([jnp.where(pr < 0.0, pr, x[0:8]), x[8:]], axis=0)
            mu = jnp.mean(x, axis=0, keepdims=True)
            st_ref[0:1, gs] = mu
            xc = xt_ref[:, gs].astype(F32) - mu
            rs = jax.lax.rsqrt(jnp.mean(xc * xc, axis=0, keepdims=True) + EPS)
            rstd[s] = rs
            st_ref[8:9, gs] = rs
            mu = jnp.where(rs < 0.0, rs, mu)
            xnt_ref[:, gs] = _pk(((xt_ref[:, gs].astype(F32) - mu) * rs).astype(BF16))

    def load_xnt(s0, s1):
        return _upk(xnt_ref[:, 128 * s0:128 * s1])

    def store_xn(s0, s1):
        xn_ref[64 * s0:64 * s1, :] = _pk(load_xnt(s0, s1).T)

    def proj_q(s0, s1):
        y = jnp.dot(_upk(wt_ref[0:D // 2, :]), load_xnt(s0, s1), preferred_element_type=F32)
        qt = _pk((y * QSCALE).astype(BF16))
        for s in range(s0, s1):
            qt_ref[s // 2, :, 128 * (s % 2):128 * (s % 2 + 1)] = qt[:, 128 * (s - s0):128 * (s - s0 + 1)]
        return y

    def proj_k(s0, s1):
        y = jnp.dot(_upk(wt_ref[D // 2:D, :]), load_xnt(s0, s1), preferred_element_type=F32)
        for s in range(s0, min(s1, NOC)):
            ktf_ref[s] = y[0:G, 128 * (s - s0):128 * (s - s0 + 1)]
        kt = _pk(y.astype(BF16))
        for g in range(4):
            lo = min(G // 2 * g, D // 2 - 64)
            k_ref[g, 64 * s0:64 * s1, :] = _pk(_upk(kt[lo:lo + 64, :]).T)
        return y

    def proj_v(s0, s1):
        y = jnp.dot(_upk(wt_ref[D:3 * D // 2, :]), load_xnt(s0, s1), preferred_element_type=F32)
        rid = jax.lax.broadcasted_iota(jnp.int32, (DP, 128 * (s1 - s0)), 0)
        for h in range(H):
            w0, v0, sp = _win(h)
            valid = (rid >= v0) & (rid < v0 + DH)
            blk = jnp.where(valid, y[w0:w0 + DP, :], jnp.where(rid == sp, 1.0, 0.0))
            vt_ref[DP // 2 * h:DP // 2 * (h + 1), 128 * s0:128 * s1] = _pk(blk.astype(BF16))
        return y

    def prep_w(c_lo, c_hi):
        for c in range(c_lo, c_hi):
            w = min(128, 3 * D - c * 128)
            wt_ref[c * 64:c * 64 + w // 2, :] = _pk(wqkv_ref[:, c * 128:c * 128 + w].T)

    def prep_wo():
        wo = wo_ref[...].astype(F32)
        rid = jax.lax.broadcasted_iota(jnp.int32, (DP, D), 0)
        blks = []
        for h in range(H):
            w0, v0, _ = _win(h)
            valid = (rid >= v0) & (rid < v0 + DH)
            blks.append(jnp.where(valid, wo[w0:w0 + DP, :], 0.0).astype(BF16))
        wot_ref[...] = _pk(jnp.concatenate(blks, axis=0).T)

    def qmask(r, h):
        g, j = divmod(h, 4)
        lo, hi = 14 * j, 14 * (j + 1)
        t0, t1 = lo // 8, -(-hi // 8)
        blk = qt_ref[r, 56 * g + 8 * t0:56 * g + 8 * t1, :]
        rid = jax.lax.broadcasted_iota(jnp.int32, blk.shape, 0) + 8 * t0
        blk = jnp.where((rid >= lo) & (rid < hi), blk, jnp.uint32(0))
        sh = 8 if g == 3 else 0
        parts = []
        if 8 * t0 + sh > 0:
            parts.append(jnp.zeros((8 * t0 + sh, TQ), U32))
        parts.append(blk)
        if 64 - 8 * t1 - sh > 0:
            parts.append(jnp.zeros((64 - 8 * t1 - sh, TQ), U32))
        return _upk(jnp.concatenate(parts, axis=0))

    def job_b(i, c, anchor, gate):
        n0 = slice(128 * i, 128 * (i + 1))
        n1 = slice(FH + 128 * i, FH + 128 * (i + 1))

        def ld(rows, cols):
            return jnp.concatenate([w1_ref[rows, cols].astype(F32), w3_ref[rows, cols].astype(F32)], axis=1)

        ra = slice(RC * c, RC * (c + 1))
        rb = slice(K0 + RC * c, K0 + RC * (c + 1))
        b11 = gate(ld(ra, n0), anchor)
        b12 = ld(ra, n1)
        if RC * c < K1:
            b21 = ld(rb, n0)
            b22 = gate(ld(rb, n1), anchor)
            ops = [b11 + b22, b12 - b22, b21 - b11, b11 + b12, b21 + b22]
        else:
            b12 = gate(b12, anchor)
            ops = [b11, b12, None, b11 + b12, None]
        for j, o in enumerate(ops):
            if o is not None:
                bo_ref[5 * i + j, ra, :] = o.astype(BF16)

    def job_a(b, c, anchor, gate):
        zpad = jnp.zeros((RC, K0 - K1), F32)
        xa = _upk(xn_ref[128 * b + RC // 2 * c:128 * b + RC // 2 * (c + 1), :]).astype(F32)
        xb = _upk(xn_ref[128 * b + 64 + RC // 2 * c:128 * b + 64 + RC // 2 * (c + 1), :]).astype(F32)
        a11, a21 = gate(xa[:, 0:K0], anchor), xb[:, 0:K0]
        a12 = jnp.concatenate([xa[:, K0:D], zpad], axis=1)
        a22 = gate(jnp.concatenate([xb[:, K0:D], zpad], axis=1), anchor)
        ops = [a11 + a22, a21 + a22, a11 + a12, a21 - a11, a12 - a22]
        for j, o in enumerate(ops):
            ao_ref[5 * b + j, RC * c:RC * (c + 1), :] = o.astype(BF16)

    def job_w2(c, half, anchor, gate):
        lo, hi = (0, 512) if half == 0 else (512, FH)
        ra = slice(8 * c, 8 * (c + 1))
        rb = slice(DH2 + 8 * c, DH2 + 8 * (c + 1))
        a11 = gate(w2t_ref[ra, lo:hi].astype(F32), anchor)
        a12 = w2t_ref[ra, FH + lo:FH + hi].astype(F32)
        a21 = w2t_ref[rb, lo:hi].astype(F32)
        a22 = gate(w2t_ref[rb, FH + lo:FH + hi].astype(F32), anchor)
        ops = [a11 + a22, a21 + a22, a11 + a12, a21 - a11, a12 - a22]
        for j, o in enumerate(ops):
            w2o_ref[j, ra, lo:hi] = o.astype(BF16)

    def job_kb(s, d, anchor, gate):
        row = gate(jnp.broadcast_to(ktf_ref[s, d:d + 1, :], (8, 128)), anchor)
        row = jnp.concatenate([row, row], axis=0).astype(BF16)
        blk = jnp.concatenate([row] * 8, axis=0).T.astype(F32)
        kb_ref[16 * s:16 * (s + 1), 8 * d:8 * (d + 1), :] = blk.reshape(16, 8, 128)

    def job_qb(b, c, anchor, gate):
        c, hf = divmod(c, 4)
        q = _upk(qt_ref[b, 8 * c:8 * (c + 1), :]).astype(F32)
        q = gate(q[8 * (hf // 2):8 * (hf // 2 + 1)], anchor)
        for i in range(4 * (hf % 2), 4 * (hf % 2 + 1)):
            d = 16 * c + 8 * (hf // 2) + i
            qb_ref[8 * d:8 * (d + 1), :] = jnp.broadcast_to(q[i:i + 1, :], (8, TQ))

    def with_jobs(projs, jobs):
        n = len(projs) * (D // 8) - 40
        k = 0
        for pi, (proj, s) in enumerate(projs):
            y = proj(s, s + 1)
            while k < len(jobs) and (k * n) // len(jobs) < (pi + 1) * (D // 8):
                row = (k * n) // len(jobs) - pi * (D // 8)
                fn, x0, x1 = jobs[k]
                fn(x0, x1, y[8 * row:8 * (row + 1), :], gate_a)
                k += 1

    def with_jobs_multi(proj, s0, s1, jobs):
        y = proj(s0, s1)
        n = (s1 - s0) * (D // 8)
        for k, (fn, x0, x1) in enumerate(jobs):
            j, row = divmod((k * n) // len(jobs), D // 8)
            fn(x0, x1, y[8 * row:8 * (row + 1), 128 * j:128 * (j + 1)], gate_a)

    def jobs_a(b0, b1):
        return [(job_a, b, c) for b in range(b0, b1) for c in range(128 // RC)]

    kbj = [(job_kb, s, d) for s in range(NOC) for d in range(G) if s < NOCS[d // DH]]
    kbs = []
    for n_ in (52, 40, 52, 76, 70, 60, 40):
        kbs.append(kbj[:n_])
        kbj = kbj[n_:]
    kbs.append(kbj)

    wait(0)
    layernorm(0, 2)
    gate_a = _gater(jnp.broadcast_to(rstd[0] < 0.0, (8, 128)))
    wait(1)
    prep_w(0, 4)
    proj_q(0, 2)
    store_xn(0, 2)
    wait(2)
    prep_w(7, 11)
    proj_v(0, 2)
    wait(3)
    prep_w(4, 7)
    layernorm(2, 5)
    proj_k(0, 2)
    with_jobs([(proj_k, s) for s in range(2, 5)], kbs[0])
    store_xn(2, 5)
    with_jobs([(proj_q, s) for s in range(2, 5)], _mix(jobs_a(0, 2), kbs[1]))
    wait(4)
    layernorm(5, 8)
    proj_v(2, 5)
    proj_q(5, 8)
    store_xn(5, 8)
    layernorm(8, 12)
    proj_k(5, 8)
    with_jobs([(proj_v, s) for s in range(5, 8)], _mix(jobs_a(2, 4), kbs[2]))
    with_jobs_multi(proj_q, 8, 12, _mix(kbs[3], [(job_qb, 1, c) for c in range(G // 4)]))
    store_xn(8, 12)
    layernorm(12, 16)
    store_xn(12, 16)
    with_jobs_multi(proj_k, 8, 12, kbs[4])
    prep_wo()
    with_jobs([(proj_v, s) for s in range(8, 12)], _mix(jobs_a(4, 8), kbs[5]))
    wait(5)
    for h in range(4):
        s0 = jnp.dot(_upk(k_ref[0, 0:NOCS[h] * CK // 2, :]), qmask(0, h), preferred_element_type=F32)
        so_ref[h, 0:NOCS[h] * CK] = s0
        om_ref[h] = jnp.max(s0.reshape(NOCS[h] * CK // 8, 8, TQ), axis=0)
        mine = kbs[6][len(kbs[6]) * sum(NOCS[:h]) // sum(NOCS):len(kbs[6]) * sum(NOCS[:h + 1]) // sum(NOCS)]
        for k, (fn, x0, x1) in enumerate(mine):
            row = k * (s0.shape[0] // 8) // len(mine)
            fn(x0, x1, s0[8 * row:8 * (row + 1), 0:128], gate_a)
    with_jobs([(p_, s) for p_ in (proj_k, proj_q, proj_v) for s in range(12, 16)],
              _mix([(job_b, i, c) for i in range(7) for c in range(K0 // RC)]
                   + [(job_w2, c, hf) for c in range(DH2 // 8) for hf in range(2)], kbs[7]))

    wait(6)

    def out_copy(r, j):
        cols = pl.ds(pl.multiple_of(r * TQ + 128 * j, 128), 128)
        return pltpu.make_async_copy(ob_ref.at[2 * r + j], o_hbm.at[:, cols], sems.at[6])

    def body(r, carry):
        zero = jnp.minimum(r, 0)
        off = pl.multiple_of(zero * 8, 8)
        gate = _gater(jax.lax.broadcasted_iota(jnp.int32, (8, 128), 1) < zero)

        qvs = [qb_ref.at[pl.ds(pl.multiple_of(jnp.minimum(r + i, 0) * 8, 8), 8 * G)] for i in range(2)]
        kbv = kb_ref.at[pl.ds(zero, NKG)]
        omv = om_ref.at[pl.ds(zero, 4)]
        part = [None]
        consumed = set()

        def score_job(h, kg, sub, anchor):
            assert h in consumed
            nd = DH // NSUB
            rows = slice(8 * (DH * h + nd * sub), 8 * (DH * h + nd * (sub + 1)))
            kb = kbv[kg, rows, :]
            kb = jax.lax.concatenate([gate(kb[0:8], anchor), kb[8:]], 0)
            t = jax.lax.concatenate([kb, kb], 1) * qvs[kg % 2][rows, :]
            u = jax.lax.concatenate([t, jnp.zeros((8, TQ), F32) if sub == 0 else part[0]], 0)
            acc = jnp.sum(jnp.sum(jnp.sum(u.reshape(2, 2, 2, 8, TQ), axis=2), axis=1), axis=0)
            part[0] = acc
            if sub == NSUB - 1:
                so_ref[h, 8 * kg:8 * (kg + 1), :] = acc
                om_ref[h] = acc if kg == 0 else jnp.maximum(omv[h], acc)

        jobs = [(h, kg, sub) for h in range(4) for kg in range(NOCS[h] * CK // 8) for sub in range(NSUB)]
        WQ, WF, WD = 80, 28, 120
        wtot = WQ * ((H - 1) * NCK - sum(NOCS[1:])) + WF * 7 * (F // 128 - 1) + WD * 6
        clock = [0]
        jdone = [0]

        def tick(y, w):
            lo = clock[0]
            clock[0] += w
            while jdone[0] < len(jobs) and (jdone[0] * wtot) // len(jobs) < clock[0]:
                row = ((jdone[0] * wtot) // len(jobs) - lo) * (y.shape[0] // 8) // w
                score_job(*jobs[jdone[0]], y[8 * row:8 * (row + 1), 0:128])
                jdone[0] += 1

        def refill_qb(y, half):
            assert jdone[0] == len(jobs)
            step = y.shape[0] // 14
            for i in range(14):
                job_qb(jnp.minimum(r + 2, NQ - 1), 14 * half + i, y[step * i:step * i + 8, :], gate)

        def qk_chunk(h, qm, c, s_ref, mrun):
            kc = _upk(k_ref[h // 4, c * CK // 2:(c + 1) * CK // 2, :])
            s = jnp.dot(kc, qm, preferred_element_type=F32)
            s_ref[c * CK:(c + 1) * CK, :] = s
            mm = jnp.max(s.reshape(CK // 8, 8, TQ), axis=0)
            mrun = mm if mrun is None else jnp.maximum(mrun, mm)
            if h >= 1:
                tick(s, WQ)
            return mrun

        def pv_chunk(h, c, s_ref, m, acc):
            if h < 4 and c < NOCS[h]:
                sv = so_ref[h, c * CK:(c + 1) * CK, :]
                if c == NOCS[h] - 1:
                    consumed.add(h)
            else:
                sv = s_ref[pl.ds(off + c * CK, CK), :]
            p = jnp.exp2(sv - m).astype(BF16)
            vc = _upk(vt_ref[DP // 2 * h:DP // 2 * (h + 1), c * CK:(c + 1) * CK])
            o = jnp.dot(vc, p, preferred_element_type=F32)
            return o if acc is None else o + acc

        def finish_pv(h, acc):
            sp = _win(h)[2]
            inv = 1.0 / acc[sp:sp + 1, :]
            ot_ref[DP // 2 * h:DP // 2 * (h + 1), :] = _pk((acc * inv).astype(BF16))

        def silu_mul(gu):
            hg = 0.5 * gu[:, 0:128]
            return (hg * jnp.tanh(hg) + hg) * gu[:, 128:256]

        def ffn_slice(f):
            i, pc = divmod(f, 2)
            n0 = slice(128 * i, 128 * (i + 1))
            n1 = slice(FH + 128 * i, FH + 128 * (i + 1))

            def asum(j, kw):
                return ao_ref[5 * r + j, 64 * pc:64 * (pc + 1), 0:kw]

            def bsum(j, kw):
                return bo_ref[5 * i + j, 0:kw, :]

            def mm(a, b):
                y = jnp.dot(a, b, preferred_element_type=F32)
                if f > 0:
                    tick(y, WF)
                return y

            a11 = _upk(xn_ref[pl.ds(pl.multiple_of(128 * r + 32 * pc, 32), 32), 0:K0])
            a22 = _upk(xn_ref[pl.ds(pl.multiple_of(128 * r + 64 + 32 * pc, 32), 32), K0:D])
            b11 = jnp.concatenate([w1_ref[0:K0, n0], w3_ref[0:K0, n0]], axis=1)
            b22 = jnp.concatenate([w1_ref[K0:D, n1], w3_ref[K0:D, n1]], axis=1)
            m1 = mm(asum(0, K0), bsum(0, K0))
            c11 = mm(asum(4, K1), bsum(4, K1)) + m1
            c22 = mm(asum(3, K0), bsum(3, K0)) + m1
            m5 = mm(asum(2, K1), b22)
            c11 = c11 - m5
            m3 = mm(a11, bsum(1, K0))
            h12 = silu_mul(m3 + m5)
            c22 = c22 + m3
            m4 = mm(a22, bsum(2, K1))
            h11 = silu_mul(c11 + m4)
            m2 = mm(asum(1, K0), b11)
            h21 = silu_mul(m2 + m4)
            h22 = silu_mul(c22 - m2)
            hops = [h11 + h22, h11, h21 - h22, h12 - h11, h22, h11 + h21, h12 + h22]
            for j, o in enumerate(hops):
                h_ref[j, 32 * pc:32 * (pc + 1), n0] = _pk(o.astype(BF16))

        def down(j):
            if j == 2:
                a = w2t_ref[0:DH2, 0:FH]
            elif j == 3:
                a = w2t_ref[DH2:D, FH:F]
            else:
                a = w2o_ref[j if j < 2 else j - 2]
            cuts = [0, 144, DH2] if j == 5 else [0, DH2]
            y = jnp.concatenate([jax.lax.dot_general(a[lo:hi], _upk(h_ref[j]), NT, preferred_element_type=F32)
                                 for lo, hi in zip(cuts[:-1], cuts[1:])], axis=0)
            if j != 5:
                tick(y, WD)
            else:
                refill_qb(y, 0)
            return y

        bufs = (sa, sb)
        m = None
        for u in range(-1, H - 1):
            hq = u + 1
            mrun = om_ref[hq] if hq < 4 else None
            acc = None
            qm = qmask(r, hq)
            for c in range(NCK):
                if not (hq < 4 and c < NOCS[hq]):
                    mrun = qk_chunk(hq, qm, c, bufs[hq % 2], mrun)
                if m is not None:
                    acc = pv_chunk(u, c, bufs[u % 2], m, acc)
            m = jnp.max(mrun, axis=0, keepdims=True)
            if acc is not None:
                finish_pv(u, acc)
            if hq < F // 128:
                ffn_slice(hq)
            elif u == H - 3:
                d4 = down(3)
            else:
                d2 = down(1)
                y21 = d2 + d4
                d5 = down(4)
                y11 = d4 - d5
        acc = None
        for t in range(4):
            for c in range(4 * t, 4 * (t + 1)):
                acc = pv_chunk(H - 1, c, bufs[(H - 1) % 2], m, acc)
            if t == 0:
                d3 = down(2)
                y12 = d3 + d5
                y22 = d3 - d2
            elif t == 1:
                d1 = down(0)
                y11 = y11 + d1
                y22 = y22 + d1
            elif t == 2:
                y11 = down(6) + y11
            else:
                finish_pv(H - 1, acc)
                y22 = down(5) + y22
        ycol = [jnp.concatenate([y11, y21], axis=0), jnp.concatenate([y12, y22], axis=0)]
        for j in range(2):
            js = slice(128 * j, 128 * (j + 1))
            yj = jnp.dot(_upk(wot_ref[...]), _upk(ot_ref[:, js]), preferred_element_type=F32) + ycol[j]
            if j == 0:
                refill_qb(yj, 1)
            ob_ref[2 * r + j] = (ob_ref[2 * r + j].astype(F32) + yj).astype(BF16)
            out_copy(r, j).start()
        return carry

    jax.lax.fori_loop(0, NQ, body, 0)
    for r in range(NQ):
        out_copy(r, 0).wait()
        out_copy(r, 1).wait()


@jax.jit
def pallas_parallel_sum__softmax_full_mha__glu_gated_swiglu__prompt_kernel(
    A_x: jax.Array,
    A_wqkv: jax.Array,
    A_wo: jax.Array,
    B_x: jax.Array,
    B_w1: jax.Array,
    B_w3: jax.Array,
    B_w2: jax.Array,
):
    del B_x
    xt = A_x.reshape(S, D).T
    any_spec = pl.BlockSpec(memory_space=pl.ANY)
    out_t = pl.pallas_call(
        _kernel,
        out_shape=jax.ShapeDtypeStruct((D, S), A_x.dtype),
        in_specs=[any_spec] * 6,
        out_specs=any_spec,
        scratch_shapes=[
            pltpu.VMEM((D, S), BF16),
            pltpu.VMEM((D, 3 * D), BF16),
            pltpu.VMEM((D, D), BF16),
            pltpu.VMEM((D, F), BF16),
            pltpu.VMEM((D, F), BF16),
            pltpu.VMEM((D, F), BF16),
            pltpu.VMEM((2 * NQ, D, 128), BF16),
            pltpu.SemaphoreType.DMA((7,)),
            pltpu.VMEM((3 * D // 2, D), U32),
            pltpu.VMEM((D // 2, H * DP), U32),
            pltpu.VMEM((S // 2, D), U32),
            pltpu.VMEM((NQ, D // 2, TQ), U32),
            pltpu.VMEM((4, S // 2, 128), U32),
            pltpu.VMEM((H * DP // 2, S), U32),
            pltpu.VMEM((S, TQ), F32),
            pltpu.VMEM((S, TQ), F32),
            pltpu.VMEM((H * DP // 2, TQ), U32),
            pltpu.VMEM((7, 64, FH), U32),
            pltpu.VMEM((D // 2, S), U32),
            pltpu.VMEM((16, S), F32),
            pltpu.VMEM((35, K0, 256), BF16),
            pltpu.VMEM((5 * NQ, 128, K0), BF16),
            pltpu.VMEM((NKG, 8 * G, 128), F32),
            pltpu.VMEM((8 * G, TQ), F32),
            pltpu.VMEM((4, NOC * CK, TQ), F32),
            pltpu.VMEM((4, 8, TQ), F32),
            pltpu.VMEM((NOC, G, 128), F32),
            pltpu.VMEM((5, D // 2, F // 2), BF16),
        ],
        compiler_params=pltpu.CompilerParams(vmem_limit_bytes=100 * 1024 * 1024),
    )(xt, A_wqkv, A_wo, B_w1, B_w3, B_w2.T)
    return out_t.T.reshape(1, S, D)
```
